```python
import os as _os
_os.environ.setdefault("JAX_PLATFORMS", "cpu")
import jax
import jax.numpy as jnp

def _softmax(x, axis=-1):
    return jax.nn.softmax(x, axis=axis)
def _gelu(x):
    return jax.nn.gelu(x, approximate=True)
def _silu(x):
    return jax.nn.silu(x)
def _sigmoid(x):
    return jax.nn.sigmoid(x)
def _layernorm(x, axis=-1, eps=1e-5):
    m = jnp.mean(x, axis=axis, keepdims=True)
    v = jnp.var(x, axis=axis, keepdims=True)
    return (x - m) / jnp.sqrt(v + eps)
def _scatter_add(tgt, idx, src, axis=0):
    return tgt.at[idx].add(src)
def _segment_sum(src, seg, n):
    return jax.ops.segment_sum(src, seg, n)
class _Rng:
    def __init__(self, key):
        self._k = key
    def _next(self):
        self._k, sub = jax.random.split(self._k)
        return sub
    def normal(self, shape):
        return jax.random.normal(self._next(), shape, dtype=jnp.bfloat16)
    def randint(self, lo, hi, shape):
        return jax.random.randint(self._next(), shape, lo, hi, dtype=jnp.int32)
    def uniform(self, shape, lo=0.0, hi=1.0):
        return jax.random.uniform(self._next(), shape, jnp.bfloat16, lo, hi)
    def permutation(self, n):
        return jax.random.permutation(self._next(), n)


kernel_name = 'concat_heads__sliding_block__ssm_conv_s4__prompt'

def setup_inputs():
    _rng = _Rng(jax.random.key(int.from_bytes(__import__("os").urandom(4), "little")))
    _w = (lambda a: (lambda t: t.astype(jnp.bfloat16) if jnp.issubdtype(t.dtype, jnp.floating) else t)(jnp.asarray(a)))
    def _A_setup():
        B, S, D = 1, 2048, 512
        return {
            "x": _w((lambda *s: _rng.normal(s) * 0.2)(B, S, D)),
            "wqkv": _w((lambda *s: _rng.normal(s) * 0.2)(D, 3 * D)),
            "wo": _w((lambda *s: _rng.normal(s) * 0.05)(D, D)),
        }
    _A_in = _A_setup()

    def _B_setup():
        B, L, D, N = 1, 2048, 512, 128
        A_re = -jnp.exp((lambda *s: _rng.normal(s) * 0.8)(D, N))
        A_im = jnp.pi * (lambda *s: _rng.normal(s) * 0.8)(D, N)
        B_re = (lambda *s: _rng.normal(s) * 0.8)(D, N)
        B_im = (lambda *s: _rng.normal(s) * 0.8)(D, N)
        C_re = (lambda *s: _rng.normal(s) * 0.8)(D, N)
        C_im = (lambda *s: _rng.normal(s) * 0.8)(D, N)
        log_dt = (lambda *s: _rng.normal(s) * 0.8)(D) * 0.5 - 4.0
        Dskip = (lambda *s: _rng.normal(s) * 0.05)(D)
        return {
            "u": _w((lambda *s: _rng.normal(s) * 0.05)(B, L, D)),
            "A_re": _w(A_re),
            "A_im": _w(A_im),
            "B_re": _w(B_re),
            "B_im": _w(B_im),
            "C_re": _w(C_re),
            "C_im": _w(C_im),
            "log_dt": _w(log_dt),
            "Dskip": _w(Dskip),
        }
    _B_in = _B_setup()

    return {
        "A_x": _A_in["x"],
        "A_wqkv": _A_in["wqkv"],
        "A_wo": _A_in["wo"],
        "B_u": _B_in["u"],
        "B_A_re": _B_in["A_re"],
        "B_A_im": _B_in["A_im"],
        "B_B_re": _B_in["B_re"],
        "B_B_im": _B_in["B_im"],
        "B_C_re": _B_in["C_re"],
        "B_C_im": _B_in["C_im"],
        "B_log_dt": _B_in["log_dt"],
        "B_Dskip": _B_in["Dskip"],
    }

def reference(A_x, A_wqkv, A_wo, B_u, B_A_re, B_A_im, B_B_re, B_B_im, B_C_re, B_C_im, B_log_dt, B_Dskip):
    def _A_ref(x, wqkv, wo):
        B, S, D = x.shape
        H = 32; Dh = D // H; W = 256
        qkv = (lambda x, *d: x.transpose(*d))((x @ wqkv).reshape(B, S, 3, H, Dh), 2, 0, 3, 1, 4)
        q, k, v = qkv[0], qkv[1], qkv[2]
        scores = jnp.einsum("bhqd,bhkd->bhqk", q, k) * (Dh ** -0.5)
        idx = jnp.arange(S)
        mask = (idx[:, None] - idx[None, :] >= 0) & (idx[:, None] - idx[None, :] < W)
        scores = jnp.where(mask[None, None], scores, -1e9)
        p = _softmax(scores, axis=-1)
        o = jnp.einsum("bhqk,bhkd->bhqd", p, v)
        return (lambda x, *d: x.transpose(*d))(o, 0, 2, 1, 3).reshape(B, S, D) @ wo

    def _B_ref(u, A_re, A_im, B_re, B_im, C_re, C_im, log_dt, Dskip):
        Bsz, L, D = u.shape
        dt = jnp.exp(log_dt)[:, None]
        A = A_re + 1j * A_im
        Bc = B_re + 1j * B_im
        Cc = C_re + 1j * C_im
        logdA = dt * A
        dB = dt * Bc
        l = (lambda x, dt: x.astype(dt))(jnp.arange(L), A_re.dtype)
        P = jnp.exp(logdA[:, :, None] * l[None, None, :])
        K = jnp.einsum("dn,dnl,dn->dl", Cc, P, dB).real
        L2 = 2 * L
        Kp = jnp.pad(K, ((0, 0), (0, L)))
        up = (lambda x, *d: x.transpose(*d))(u, 0, 2, 1)
        up = jnp.pad(up, ((0, 0), (0, 0), (0, L)))
        Kf = (lambda x, axes=(-2,-1): jnp.fft.rfft2(x.astype(jnp.float32), axes=axes))(Kp[:, None, :], axes=(-2, -1))
        Uf = (lambda x, axes=(-2,-1): jnp.fft.rfft2(x.astype(jnp.float32), axes=axes))(up[:, :, None, :], axes=(-2, -1))
        Yf = Uf * Kf[None, :, :, :]
        y = (lambda x, s, axes=(-2,-1): jnp.fft.irfft2(x, s=s, axes=axes).astype(jnp.bfloat16))(Yf, (1, L2), axes=(-2, -1))[:, :, 0, :L]
        y = (lambda x, *d: x.transpose(*d))(y, 0, 2, 1) + u * Dskip[None, None, :]
        return y

    a = _A_ref(A_x, A_wqkv, A_wo)
    b = _B_ref(B_u, B_A_re, B_A_im, B_B_re, B_B_im, B_C_re, B_C_im, B_log_dt, B_Dskip)
    return jnp.concatenate([a, b], axis=-1)
```

```python
import math

import numpy as np
import jax
import jax.numpy as jnp
import jax.experimental.pallas as pl
import jax.experimental.pallas.tpu as pltpu

F32 = jnp.float32
BF16 = jnp.bfloat16

S = 2048
D = 512
NEG = -1e30
RB = 512
NKB = 18


def _part_a(x_ref, wqkv_ref, wo_ref, out_store, qs, km, vt, ob):
    lane = jax.lax.broadcasted_iota(jnp.int32, (128, 128), 1)
    row = jax.lax.broadcasted_iota(jnp.int32, (128, 128), 0)
    zeros_k = jnp.zeros((8 * 128, 128), BF16)
    for g in range(4):
        for jb in range(2):
            km[pl.ds(((g * NKB + jb) * 8) * 128, 1024), :] = zeros_k
    vt[:, 0:256] = jnp.zeros((512, 256), BF16)
    for r0 in range(0, S, RB):
        xb = x_ref[r0:r0 + RB, :]
        q = jnp.dot(xb, wqkv_ref[:, 0:512], preferred_element_type=F32).astype(BF16)
        qs[r0:r0 + RB, :] = q * jnp.asarray(0.25, BF16)
        k = jnp.dot(xb, wqkv_ref[:, 512:1024], preferred_element_type=F32).astype(BF16)
        for g in range(4):
            for bb in range(RB // 128):
                kb = k[128 * bb:128 * (bb + 1), 128 * g:128 * (g + 1)]
                jb = (r0 // 128) + bb + 2
                for hh in range(8):
                    msk = (lane >= 16 * hh) & (lane < 16 * (hh + 1))
                    km[pl.ds(((g * NKB + jb) * 8 + hh) * 128, 128), :] = jnp.where(msk, kb, jnp.zeros_like(kb))
        v_t = jax.lax.dot_general(wqkv_ref[:, 1024:1536], xb, (((0,), (1,)), ((), ())),
                                  preferred_element_type=F32)
        vt[:, 256 + r0:256 + r0 + RB] = v_t.astype(BF16)

    tri = row <= lane

    def item(it, c):
        g = it // 16
        i = it % 16
        q0 = pl.multiple_of(i * 128, 128)
        g0 = pl.multiple_of(g * 128, 128)
        qi = qs[pl.ds(q0, 128), pl.ds(g0, 128)]
        kstart = pl.multiple_of((g * NKB + i) * 1024, 1024)
        kw = km[pl.ds(kstart, 3072), :]
        st_all = jax.lax.dot_general(kw, qi, (((1,), (1,)), ((), ())), preferred_element_type=F32)
        v0 = i >= 2
        v1 = i >= 1
        ots = []
        for hh in range(8):
            s0 = st_all[(0 + hh) * 128:(0 + hh) * 128 + 128]
            s1 = st_all[(8 + hh) * 128:(8 + hh) * 128 + 128]
            s2 = st_all[(16 + hh) * 128:(16 + hh) * 128 + 128]
            sm = jnp.where(tri, s2, jnp.where(v0, s0, NEG))
            s1 = jnp.where(v1, s1, NEG)
            m = jnp.maximum(jnp.max(sm, axis=0, keepdims=True), jnp.max(s1, axis=0, keepdims=True))
            pm = jnp.exp(sm - m)
            p1 = jnp.exp(s1 - m)
            l = jnp.sum(pm, axis=0, keepdims=True) + jnp.sum(p1, axis=0, keepdims=True)
            p2 = jnp.where(tri, pm, 0.0)
            p0 = jnp.where(tri, 0.0, pm)
            pt = jnp.concatenate([p0.astype(BF16), p1.astype(BF16), p2.astype(BF16)], axis=0)
            e0 = pl.multiple_of(g * 128 + hh * 16, 16)
            vtw = vt[pl.ds(e0, 16), pl.ds(q0, 384)]
            ot = jnp.dot(vtw, pt, preferred_element_type=F32)
            ots.append(ot / l)
        otb = jnp.concatenate(ots, axis=0)
        ob[pl.ds(q0, 128), pl.ds(g0, 128)] = otb.T.astype(BF16)
        return c

    jax.lax.fori_loop(0, 64, item, 0)
    for r0 in range(0, S, RB):
        o = jnp.dot(ob[r0:r0 + RB, :], wo_ref[...], preferred_element_type=F32)
        out_store(r0, RB, o.astype(BF16))


L = 2048


def _exp_acc(x):
    x = jnp.maximum(x, -87.0)
    k = jnp.floor(x * 1.44269504088896341 + 0.5)
    r = x - k * 0.693359375
    r = r - k * (-2.12194440e-4)
    p = 1.9875691500e-4
    for cf in (1.3981999507e-3, 8.3334519073e-3, 4.1665795894e-2, 1.6666665459e-1, 5.0000001201e-1):
        p = p * r + cf
    p = p * (r * r) + r + 1.0
    ki = k.astype(jnp.int32)
    sc = jax.lax.bitcast_convert_type((ki + 127) << 23, F32)
    return p * sc


def _sincos_acc(t):
    k = jnp.floor(t * 0.636619772367581343 + 0.5)
    r = t - k * 1.5703125
    r = r - k * 4.837512969970703125e-4
    r = r - k * 7.54978995489188216e-8
    r2 = r * r
    s = ((-1.9515295891e-4 * r2 + 8.3321608736e-3) * r2 + (-1.6666654611e-1)) * (r2 * r) + r
    c = ((2.443315711809948e-5 * r2 + (-1.388731625493765e-3)) * r2 + 4.166664568298827e-2) * (r2 * r2) \
        - 0.5 * r2 + 1.0
    q = k.astype(jnp.int32) & 3
    swap = (q & 1) == 1
    sn = jnp.where(swap, c, s)
    cs = jnp.where(swap, s, c)
    sn = jnp.where(q >= 2, -sn, sn)
    cs = jnp.where((q == 1) | (q == 2), -cs, cs)
    return sn, cs


def _cexp(xr, xi):
    e = _exp_acc(xr)
    s, c = _sincos_acc(xi)
    return e * c, e * s


def _cmul_const(xr, xi, wr, wi):
    eps = 1e-12
    if abs(wi) < eps:
        if abs(wr - 1) < eps:
            return xr, xi
        if abs(wr + 1) < eps:
            return -xr, -xi
    if abs(wr) < eps:
        if abs(wi - 1) < eps:
            return -xi, xr
        if abs(wi + 1) < eps:
            return xi, -xr
    if abs(abs(wr) - abs(wi)) < eps:
        s = abs(wr)
        a = 1.0 if wr > 0 else -1.0
        b = 1.0 if wi > 0 else -1.0
        if a * b > 0:
            return (xr - xi) * (a * s), (xr + xi) * (a * s)
        return (xr + xi) * (a * s), (xr - xi) * (-a * s)
    return xr * wr - xi * wi, xr * wi + xi * wr


def _dft(xs, sign):
    n = len(xs)
    if n == 1:
        return xs
    ev = _dft(xs[0::2], sign)
    od = _dft(xs[1::2], sign)
    out = [None] * n
    for k in range(n // 2):
        ang = sign * 2 * math.pi * k / n
        tr, ti = _cmul_const(od[k][0], od[k][1], math.cos(ang), math.sin(ang))
        er, ei = ev[k]
        out[k] = (er + tr, ei + ti)
        out[k + n // 2] = (er - tr, ei - ti)
    return out


A_RE, A_IM = 0, 2048
B_RE, B_IM = 4096, 6144
SEED_RE = 8192
SEED_IM = SEED_RE + 768
C_RE = SEED_RE + 1536
C_IM = C_RE + 64
PAR = C_RE + 128
NPOOL = PAR + 384
E_RE, E_IM = 4096, 4096 + 1024
G_RE, G_IM = 4096 + 2048, 4096 + 2048 + 1088
TWN = 4096


def _part_b(u_ref, are_ref, aim_ref, bre_ref, bim_ref, cre_ref, cim_ref, ldt_ref, dsk_ref, tw_ref,
            out_store, pool, ubuf, ybuf):
    def ld(i):
        return pool[pl.ds(pl.multiple_of(i * 8, 8), 8), :]

    def st(i, v):
        pool[pl.ds(pl.multiple_of(i * 8, 8), 8), :] = v

    def swaph(v):
        return pltpu.roll(v, 4, 0)

    for a_i, ref in enumerate((are_ref, aim_ref, bre_ref, bim_ref, cre_ref, cim_ref)):
        for g in range(4):
            blk = ref[128 * g:128 * (g + 1), :].astype(F32)
            pool[pl.ds((PAR + a_i * 64) * 8 + g, 128, stride=4), :] = blk.T
    dt4 = _exp_acc(ldt_ref[...].astype(F32)).astype(BF16).astype(F32)
    dt8 = jnp.concatenate([dt4, dt4], axis=0)

    for g in range(4):
        for r0 in range(0, L, 256):
            ubuf[g * L + r0:g * L + r0 + 256, :] = u_ref[r0:r0 + 256, 128 * g:128 * (g + 1)].astype(F32)

    def u_relayout(j, c):
        for g in range(4):
            ev = ubuf[pl.ds(g * L + 16 * j, 8, stride=2), :]
            od = ubuf[pl.ds(g * L + 16 * j + 1, 8, stride=2), :]
            pool[pl.ds((A_RE + 8 * j) * 8 + g, 8, stride=8), :] = ev
            pool[pl.ds((A_IM + 8 * j) * 8 + g, 8, stride=8), :] = od
        return c
    jax.lax.fori_loop(0, 128, u_relayout, 0)

    kscale = 2.0 ** -14

    def seeds(np_, c):
        ar = dt8 * ld(PAR + 0 * 64 + np_)
        ai = dt8 * ld(PAR + 1 * 64 + np_)
        dbr = dt8 * ld(PAR + 2 * 64 + np_)
        dbi = dt8 * ld(PAR + 3 * 64 + np_)
        cr = ld(PAR + 4 * 64 + np_)
        ci = ld(PAR + 5 * 64 + np_)
        st(C_RE + np_, (cr * dbr - ci * dbi) * kscale)
        st(C_IM + np_, (cr * dbi + ci * dbr) * kscale)
        for q0, mult in ((0, 1.0), (6, 64.0)):
            zr, zi = _cexp(ar * mult, ai * mult)
            for q in range(q0, q0 + 6):
                st(SEED_RE + q * 64 + np_, zr)
                st(SEED_IM + q * 64 + np_, zi)
                if q < q0 + 5:
                    zr, zi = zr * zr - zi * zi, 2.0 * (zr * zi)
        return c
    jax.lax.fori_loop(0, 64, seeds, 0, unroll=2)

    def cmul(ar, ai, br, bi):
        return ar * br - ai * bi, ar * bi + ai * br

    def sd(q, np_):
        return ld(SEED_RE + q * 64 + np_), ld(SEED_IM + q * 64 + np_)

    def st_k(t_par, m, v):
        base = A_IM if t_par else A_RE
        pool[pl.ds(pl.multiple_of((base + m) * 8, 8) + 4, 4), :] = v[4:8]

    for s in (3, 2, 1, 0):
        sig = 1 << s
        blocks = [(0, 0), (1, 128)] if s == 0 else [(0, 128)]
        nj1 = 9 if s == 3 else 8

        def tables(np_, c, s=s, blocks=blocks, nj1=nj1):
            ev = [None] * 16
            ev[0] = (jnp.ones((8, 128), F32), jnp.zeros((8, 128), F32))
            for j0 in range(1, 16):
                hb = 1 << (j0.bit_length() - 1)
                sq = sd(s + hb.bit_length() - 1, np_)
                ev[j0] = sq if j0 == hb else cmul(*ev[j0 - hb], *sq)
            for j0 in range(16):
                st(E_RE + np_ * 16 + j0, ev[j0][0])
                st(E_IM + np_ * 16 + j0, ev[j0][1])
            c0 = (ld(C_RE + np_), ld(C_IM + np_))
            for bslot, off in blocks:
                gv = [None] * nj1
                gv[0] = c0 if off == 0 else cmul(*c0, *sd(s + 7, np_))
                for j1 in range(1, nj1):
                    hb = 1 << (j1.bit_length() - 1)
                    gv[j1] = cmul(*gv[j1 - hb], *sd(s + 4 + hb.bit_length() - 1, np_))
                for j1 in range(nj1):
                    st(G_RE + (bslot * 8 + j1) * 64 + np_, gv[j1][0])
                    st(G_IM + (bslot * 8 + j1) * 64 + np_, gv[j1][1])
            return c
        jax.lax.fori_loop(0, 64, tables, 0)

        def item(it, c, s=s, sig=sig):
            def body(np_, acc):
                er = pool[pl.ds(pl.multiple_of((E_RE + np_ * 16) * 8, 8), 128), :].reshape(16, 8, 128)
                ei = pool[pl.ds(pl.multiple_of((E_IM + np_ * 16) * 8, 8), 128), :].reshape(16, 8, 128)
                gr = ld(G_RE + it * 64 + np_)
                gi = ld(G_IM + it * 64 + np_)
                return acc + (gr[None] * er - gi[None] * ei)
            acc = jax.lax.fori_loop(0, 64, body, jnp.zeros((16, 8, 128), F32), unroll=16)
            l0 = 16 * it if s == 0 else sig * (128 + 16 * it)
            h0 = l0 // 2
            for j0 in range(16):
                v = acc[j0]
                v = v + swaph(v)
                if sig == 1:
                    box = (0,)
                elif j0 % 2 == 0:
                    box = tuple(range(-(sig // 2), sig // 2 + 1))
                else:
                    box = tuple(range(-(sig // 2) + 1, sig // 2))
                for dlt in box:
                    t_off = sig * j0 + dlt
                    st_k(t_off & 1, h0 + (t_off >> 1), v)
            return c
        jax.lax.fori_loop(0, 16 if s == 0 else 8, item, 0)

        if s == 3:
            def body2048(np_, acc):
                gr = ld(G_RE + 8 * 64 + np_)
                gi = ld(G_IM + 8 * 64 + np_)
                del gi
                return acc + gr
            acc = jax.lax.fori_loop(0, 64, body2048, jnp.zeros((8, 128), F32), unroll=8)
            v = acc + swaph(acc)
            for t in range(2044, 2048):
                st_k(t & 1, t >> 1, v)

    def tw(e):
        return tw_ref[0, e], -tw_ref[1, e]

    def fwd1(n2, c):
        xs = [(ld(A_RE + 32 * n1 + n2), ld(A_IM + 32 * n1 + n2)) for n1 in range(32)]
        for br in range(2):
            if br == 1:
                xs2 = []
                for n1 in range(32):
                    wr, wi = tw(2 * (32 * n1 + n2))
                    xr, xi = xs[n1]
                    xs2.append((xr * wr - xi * wi, xr * wi + xi * wr))
            else:
                xs2 = xs
            ys = _dft(xs2, -1)
            for k1 in range(32):
                yr, yi = ys[k1]
                if k1 > 0:
                    wr, wi = tw(4 * k1 * n2)
                    yr, yi = yr * wr - yi * wi, yr * wi + yi * wr
                st(B_RE + br * 1024 + k1 * 32 + n2, yr)
                st(B_IM + br * 1024 + k1 * 32 + n2, yi)
        return c
    jax.lax.fori_loop(0, 32, fwd1, 0)

    def fwd2(gk, c):
        br = gk // 32
        k1 = gk % 32
        xs = [(ld(B_RE + gk * 32 + n2), ld(B_IM + gk * 32 + n2)) for n2 in range(32)]
        ys = _dft(xs, -1)
        for k2 in range(32):
            k = 2 * (k1 + 32 * k2) + br
            st(A_RE + k, ys[k2][0])
            st(A_IM + k, ys[k2][1])
        return c
    jax.lax.fori_loop(0, 64, fwd2, 0)

    M = 2048

    def post(k2, c):
        for par in range(2):
            k = 2 * k2 + par
            kb = (M - k) & (M - 1)
            ar, ai = ld(A_RE + k), ld(A_IM + k)
            br_, bi_ = ld(A_RE + kb), ld(A_IM + kb)
            wr, wi = tw(k)
            er = ar + br_
            ei = ai - bi_
            dr = ar - br_
            di = ai + bi_
            tr = wr * di + wi * dr
            ti = wi * di - wr * dr
            x1r, x1i = er + tr, ei + ti
            x2r, x2i = er - tr, ti - ei
            r1r, r1i = swaph(x1r), swaph(x1i)
            r2r, r2i = swaph(x2r), swaph(x2i)
            y1r = x1r * r1r - x1i * r1i
            y1i = x1r * r1i + x1i * r1r
            y2r = x2r * r2r - x2i * r2i
            y2i = x2r * r2i + x2i * r2r
            yer = y1r + y2r
            yei = y1i - y2i
            qr = y1r - y2r
            qi = y1i + y2i
            yor = qr * wr + qi * wi
            yoi = qi * wr - qr * wi
            z1r = yer - yoi
            z1i = yei + yor
            z2r = yer + yoi
            z2i = yor - yei
            q1 = k2
            q2 = (1024 - k2) if par == 0 else (1023 - k2)
            lo = 4 * par
            for q, vr, vi in ((q1, z1r, z1i), (q2, z2r, z2i)):
                qq = jnp.where(q > 1023, 0, q) if par == 0 else q
                pool[pl.ds(pl.multiple_of((B_RE + qq) * 8, 8) + lo, 4), :] = vr[lo:lo + 4]
                pool[pl.ds(pl.multiple_of((B_IM + qq) * 8, 8) + lo, 4), :] = vi[lo:lo + 4]
        return c
    jax.lax.fori_loop(0, 513, post, 0)

    def inv1(n2, c):
        xs = [(ld(B_RE + 32 * n1 + n2), ld(B_IM + 32 * n1 + n2)) for n1 in range(32)]
        ys = _dft(xs, +1)
        for k1 in range(32):
            yr, yi = ys[k1]
            if k1 > 0:
                wr, wi = tw(4 * k1 * n2)
                wi = -wi
                yr, yi = yr * wr - yi * wi, yr * wi + yi * wr
            st(A_RE + k1 * 32 + n2, yr)
            st(A_IM + k1 * 32 + n2, yi)
        return c
    jax.lax.fori_loop(0, 32, inv1, 0)

    def inv2(k1, c):
        xs = [(ld(A_RE + k1 * 32 + n2), ld(A_IM + k1 * 32 + n2)) for n2 in range(32)]
        ys = _dft(xs, +1)
        for k2 in range(32):
            st(B_RE + k1 + 32 * k2, ys[k2][0])
            st(B_IM + k1 + 32 * k2, ys[k2][1])
        return c
    jax.lax.fori_loop(0, 32, inv2, 0)

    def comb(m, c):
        vr, vi = ld(B_RE + m), ld(B_IM + m)
        wr, wi = tw(2 * m)
        wi = -wi
        rr, ri = swaph(vr), swaph(vi)
        st(A_RE + m, vr + (rr * wr - ri * wi))
        st(A_IM + m, vi + (rr * wi + ri * wr))
        return c
    jax.lax.fori_loop(0, 1024, comb, 0, unroll=4)

    def y_relayout(j, c):
        for g in range(4):
            ev = pool[pl.ds((A_RE + 8 * j) * 8 + g, 8, stride=8), :]
            od = pool[pl.ds((A_IM + 8 * j) * 8 + g, 8, stride=8), :]
            ybuf[pl.ds(g * L + 16 * j, 8, stride=2), :] = ev
            ybuf[pl.ds(g * L + 16 * j + 1, 8, stride=2), :] = od
        return c
    jax.lax.fori_loop(0, 128, y_relayout, 0)
    for g in range(4):
        dsk = dsk_ref[:, 128 * g:128 * (g + 1)].astype(F32)
        for r0 in range(0, L, 256):
            yb = ybuf[g * L + r0:g * L + r0 + 256, :].astype(BF16).astype(F32)
            sk = (ubuf[g * L + r0:g * L + r0 + 256, :] * dsk).astype(BF16).astype(F32)
            out_store(r0, 256, g, (yb + sk).astype(BF16))


def _tw_table():
    e = np.arange(TWN)
    return np.stack([np.cos(2 * np.pi * e / TWN), np.sin(2 * np.pi * e / TWN)]).astype(np.float32)


def _kernel(tw_ref, x_ref, wqkv_ref, wo_ref, u_ref, are_ref, aim_ref, bre_ref, bim_ref, cre_ref, cim_ref,
            ldt_ref, dsk_ref, o_ref, qs, km, vt, ob, pool, ubuf, ybuf):
    def store_a(r0, n, v):
        o_ref[r0:r0 + n, 0:512] = v

    def store_b(r0, n, g, v):
        o_ref[r0:r0 + n, 512 + 128 * g:512 + 128 * (g + 1)] = v

    _part_a(x_ref, wqkv_ref, wo_ref, store_a, qs, km, vt, ob)
    _part_b(u_ref, are_ref, aim_ref, bre_ref, bim_ref, cre_ref, cim_ref, ldt_ref, dsk_ref, tw_ref,
            store_b, pool, ubuf, ybuf)


@jax.jit
def pallas_concat_heads__sliding_block__ssm_conv_s4__prompt_kernel(
    A_x: jax.Array,
    A_wqkv: jax.Array,
    A_wo: jax.Array,
    B_u: jax.Array,
    B_A_re: jax.Array,
    B_A_im: jax.Array,
    B_B_re: jax.Array,
    B_B_im: jax.Array,
    B_C_re: jax.Array,
    B_C_im: jax.Array,
    B_log_dt: jax.Array,
    B_Dskip: jax.Array,
):
    vm = pl.BlockSpec(memory_space=pltpu.VMEM)
    out = pl.pallas_call(
        _kernel,
        out_shape=jax.ShapeDtypeStruct((S, 2 * D), BF16),
        in_specs=[pl.BlockSpec(memory_space=pltpu.SMEM)] + [vm] * 12,
        out_specs=vm,
        scratch_shapes=[
            pltpu.VMEM((S, D), BF16),
            pltpu.VMEM((4 * NKB * 8 * 128, 128), BF16),
            pltpu.VMEM((512, 256 + S), BF16),
            pltpu.VMEM((S, D), BF16),
            pltpu.VMEM((NPOOL * 8, 128), F32),
            pltpu.VMEM((4 * L, 128), F32),
            pltpu.VMEM((4 * L, 128), F32),
        ],
        compiler_params=pltpu.CompilerParams(vmem_limit_bytes=120 * 1024 * 1024),
    )(jnp.asarray(_tw_table()), A_x.reshape(S, D), A_wqkv, A_wo, B_u.reshape(L, D),
      B_A_re, B_A_im, B_B_re, B_B_im, B_C_re, B_C_im, B_log_dt.reshape(4, 128), B_Dskip.reshape(1, D))
    return out.reshape(1, S, 2 * D)
```

```python
import math

import numpy as np
import jax
import jax.numpy as jnp
import jax.experimental.pallas as pl
import jax.experimental.pallas.tpu as pltpu

F32 = jnp.float32
BF16 = jnp.bfloat16

S = 2048
D = 512
L = 2048
NEG = -1e30
NKB = 18
QRB = 256
UPI = 4


def _exp_acc(x):
    x = jnp.maximum(x, -87.0)
    k = jnp.floor(x * 1.44269504088896341 + 0.5)
    r = x - k * 0.693359375
    r = r - k * (-2.12194440e-4)
    p = 1.9875691500e-4
    for cf in (1.3981999507e-3, 8.3334519073e-3, 4.1665795894e-2, 1.6666665459e-1, 5.0000001201e-1):
        p = p * r + cf
    p = p * (r * r) + r + 1.0
    ki = k.astype(jnp.int32)
    sc = jax.lax.bitcast_convert_type((ki + 127) << 23, F32)
    return p * sc


def _sincos_acc(t):
    k = jnp.floor(t * 0.636619772367581343 + 0.5)
    r = t - k * 1.5703125
    r = r - k * 4.837512969970703125e-4
    r = r - k * 7.54978995489188216e-8
    r2 = r * r
    s = ((-1.9515295891e-4 * r2 + 8.3321608736e-3) * r2 + (-1.6666654611e-1)) * (r2 * r) + r
    c = ((2.443315711809948e-5 * r2 + (-1.388731625493765e-3)) * r2 + 4.166664568298827e-2) * (r2 * r2) \
        - 0.5 * r2 + 1.0
    q = k.astype(jnp.int32) & 3
    swap = (q & 1) == 1
    sn = jnp.where(swap, c, s)
    cs = jnp.where(swap, s, c)
    sn = jnp.where(q >= 2, -sn, sn)
    cs = jnp.where((q == 1) | (q == 2), -cs, cs)
    return sn, cs


def _cexp(xr, xi):
    e = _exp_acc(xr)
    s, c = _sincos_acc(xi)
    return e * c, e * s


def _cmul_const(xr, xi, wr, wi):
    eps = 1e-12
    if abs(wi) < eps:
        if abs(wr - 1) < eps:
            return xr, xi
        if abs(wr + 1) < eps:
            return -xr, -xi
    if abs(wr) < eps:
        if abs(wi - 1) < eps:
            return -xi, xr
        if abs(wi + 1) < eps:
            return xi, -xr
    if abs(abs(wr) - abs(wi)) < eps:
        s = abs(wr)
        a = 1.0 if wr > 0 else -1.0
        b = 1.0 if wi > 0 else -1.0
        if a * b > 0:
            return (xr - xi) * (a * s), (xr + xi) * (a * s)
        return (xr + xi) * (a * s), (xr - xi) * (-a * s)
    return xr * wr - xi * wi, xr * wi + xi * wr


def _dft(xs, sign):
    n = len(xs)
    if n == 1:
        return xs
    ev = _dft(xs[0::2], sign)
    od = _dft(xs[1::2], sign)
    out = [None] * n
    for k in range(n // 2):
        ang = sign * 2 * math.pi * k / n
        tr, ti = _cmul_const(od[k][0], od[k][1], math.cos(ang), math.sin(ang))
        er, ei = ev[k]
        out[k] = (er + tr, ei + ti)
        out[k + n // 2] = (er - tr, ei - ti)
    return out


A_RE, A_IM = 0, 2048
B_RE, B_IM = 0, 2048
SEED_RE = 0
SEED_IM = SEED_RE + 768
C_RE = SEED_RE + 1536
C_IM = C_RE + 64
NSEED = C_RE + 128
E_RE, E_IM = 0, 1024
G_RE, G_IM = 2048, 2048 + 1088
ACC = G_IM + 1088
NTAB = ACC + 1024
TWN = 4096


def _tw_table():
    e = np.arange(TWN)
    return np.stack([np.cos(2 * np.pi * e / TWN), np.sin(2 * np.pi * e / TWN)]).astype(np.float32)


def _kernel(tw_ref, x_ref, wqkv_ref, wo_ref, u_ref, are_ref, aim_ref, bre_ref, bim_ref, cre_ref, cim_ref,
            ldt_ref, dsk_ref, o_ref, qs, km, vtx, ob, pa, pb, ps, ptab, ppar, ubuf, ybuf):
    lane = jax.lax.broadcasted_iota(jnp.int32, (128, 128), 1)
    row = jax.lax.broadcasted_iota(jnp.int32, (128, 128), 0)
    tri = row <= lane

    def qkv_phase():
        RB = 512
        for r0 in range(0, S, RB):
            xb = x_ref[r0:r0 + RB, :]
            q = jnp.dot(xb, wqkv_ref[:, 0:512], preferred_element_type=F32).astype(BF16)
            qs[r0:r0 + RB, :] = q * jnp.asarray(0.25, BF16)
            k = jnp.dot(xb, wqkv_ref[:, 512:1024], preferred_element_type=F32).astype(BF16)
            for g in range(4):
                for bb in range(RB // 128):
                    kb = k[128 * bb:128 * (bb + 1), 128 * g:128 * (g + 1)]
                    jb = (r0 // 128) + bb + 2
                    for hh in range(8):
                        msk = (lane >= 16 * hh) & (lane < 16 * (hh + 1))
                        km[pl.ds(((g * NKB + jb) * 8 + hh) * 128, 128), :] = jnp.where(msk, kb, jnp.zeros_like(kb))
            v_t = jax.lax.dot_general(wqkv_ref[:, 1024:1536], xb, (((0,), (1,)), ((), ())),
                                      preferred_element_type=F32).astype(BF16)
            for h in range(32):
                vtx[h * 32:h * 32 + 16, 256 + r0:256 + r0 + RB] = v_t[16 * h:16 * (h + 1)]

    def decode(a):
        lo = a < 8
        r = a - 8
        g = jnp.where(lo, a // 2, r // 14)
        i = jnp.where(lo, a % 2, 2 + r % 14)
        return g, i

    def item8(a, masked):
        g, i = decode(a)
        q0 = pl.multiple_of(i * 128, 128)
        g0 = pl.multiple_of(g * 128, 128)
        qi = qs[pl.ds(q0, 128), pl.ds(g0, 128)]
        kw = km[pl.ds(pl.multiple_of((g * NKB + i) * 1024, 1024), 3072), :]
        st_all = jax.lax.dot_general(kw, qi, (((1,), (1,)), ((), ())), preferred_element_type=F32)
        for hh in range(8):
            s0 = st_all[(0 + hh) * 128:(0 + hh) * 128 + 128]
            s1 = st_all[(8 + hh) * 128:(8 + hh) * 128 + 128]
            s2 = st_all[(16 + hh) * 128:(16 + hh) * 128 + 128]
            if masked:
                s0 = jnp.where(i >= 2, s0, NEG)
                s1 = jnp.where(i >= 1, s1, NEG)
            sm = jnp.where(tri, s2, s0)
            m = jnp.maximum(jnp.max(sm, axis=0, keepdims=True), jnp.max(s1, axis=0, keepdims=True))
            pm = jnp.exp(sm - m)
            p1 = jnp.exp(s1 - m)
            pt = jnp.concatenate([jnp.where(tri, 0.0, pm), p1, jnp.where(tri, pm, 0.0)], axis=0).astype(BF16)
            h = g * 8 + hh
            vtw = vtx[pl.ds(pl.multiple_of(h * 32, 32), 32), pl.ds(q0, 384)]
            ot = jnp.dot(vtw, pt, preferred_element_type=F32)
            ob[pl.ds(pl.multiple_of(h * 16, 16), 16), pl.ds(q0, 128)] = (ot[0:16] / ot[16:17]).astype(BF16)

    def a_unit_m(a):
        item8(a, True)

    def a_unit_f(a):
        item8(a, False)

    def o_unit(j):
        r0 = pl.multiple_of(j * QRB, QRB)
        o = jax.lax.dot_general(ob[:, pl.ds(r0, QRB)], wo_ref[...], (((0,), (0,)), ((), ())),
                                preferred_element_type=F32)
        o_ref[pl.ds(r0, QRB), 0:512] = o.astype(BF16)

    mxu_fns = {'am': a_unit_m, 'af': a_unit_f}
    mxu_q = [['am', 0, 8], ['af', 8, 56]]

    def a_prologue():
        stage_a(0)
        stage_b(0, True)
        stage_a(1)

    def a_epilogue():
        stage_c(510)
        stage_b(511, False)
        stage_c(511)

    def next_mxu():
        while mxu_q and mxu_q[0][0] in ('pro', 'epi'):
            kind = mxu_q.pop(0)[0]
            a_prologue() if kind == 'pro' else a_epilogue()
        return mxu_q[0] if mxu_q else None

    carry_units = []

    def run_vpu(name, fn, n, upi_a):
        done = 0
        while done < n:
            seg = next_mxu()
            if seg is None:
                cnt = n - done
                base_v = done
                with jax.named_scope('V_' + name):
                    jax.lax.fori_loop(0, cnt, lambda j, c, base_v=base_v: (fn(base_v + j), c)[1], 0)
                done += cnt
                continue
            kind, start, left = seg
            upi = upi_a
            rem = n - done
            if rem < upi:
                base_v = done
                with jax.named_scope('V_' + name):
                    jax.lax.fori_loop(0, rem, lambda j, c, base_v=base_v: (fn(base_v + j), c)[1], 0)
                done += rem
                continue
            cnt = min(rem // upi, left)
            base_v, base_m, mf = done, start, mxu_fns[kind]

            def body(j, c, base_v=base_v, base_m=base_m, mf=mf, upi=upi):
                mf(base_m + j)
                for q in range(upi):
                    fn(base_v + j * upi + q)
                return c
            with jax.named_scope('F_' + name + '_' + kind):
                jax.lax.fori_loop(0, cnt, body, 0)
            seg[1] += cnt
            seg[2] -= cnt
            if seg[2] == 0:
                mxu_q.pop(0)
            done += cnt * upi

    def flush_mxu():
        while True:
            seg = next_mxu()
            if seg is None:
                break
            kind, start, left = seg
            mf = mxu_fns[kind]
            with jax.named_scope('M_' + kind):
                jax.lax.fori_loop(0, left, lambda j, c, start=start, mf=mf: (mf(start + j), c)[1], 0)
            mxu_q.pop(0)

    def ld(ref, i):
        return ref[pl.ds(pl.multiple_of(i * 8, 8), 8), :]

    def st(ref, i, v):
        ref[pl.ds(pl.multiple_of(i * 8, 8), 8), :] = v

    def swaph(v):
        return pltpu.roll(v, 4, 0)

    def cmul(ar, ai, br, bi):
        return ar * br - ai * bi, ar * bi + ai * br

    def sd(q, np_):
        return ld(ps, SEED_RE + q * 64 + np_), ld(ps, SEED_IM + q * 64 + np_)

    def st_k(t_par, m, v):
        base = A_IM if t_par else A_RE
        pa[pl.ds(pl.multiple_of((base + m) * 8, 8) + 4, 4), :] = v[4:8]

    def tw(e):
        return tw_ref[0, e], -tw_ref[1, e]

    zk = jnp.zeros((2048, 128), BF16)
    for g in range(4):
        km[pl.ds((g * NKB) * 1024, 2048), :] = zk
    r32 = jax.lax.broadcasted_iota(jnp.int32, (16, 256 + S), 0)
    ones_blk = jnp.where(r32 == 0, 1.0, 0.0).astype(BF16)
    for h in range(32):
        vtx[pl.ds(h * 32 + 16, 16), :] = ones_blk
        vtx[pl.ds(h * 32, 16), 0:256] = jnp.zeros((16, 256), BF16)

    with jax.named_scope('QKV'):
        qkv_phase()

    with jax.named_scope('B0'):
        for a_i, ref in enumerate((are_ref, aim_ref, bre_ref, bim_ref, cre_ref, cim_ref)):
            for g in range(4):
                blk = ref[128 * g:128 * (g + 1), :].astype(F32)
                ppar[pl.ds((a_i * 64) * 8 + g, 128, stride=4), :] = blk.T
        dt4 = _exp_acc(ldt_ref[...].astype(F32)).astype(BF16).astype(F32)
        dt8 = jnp.concatenate([dt4, dt4], axis=0)
        for g in range(4):
            for r0 in range(0, L, 256):
                ubuf[g * L + r0:g * L + r0 + 256, :] = u_ref[r0:r0 + 256, 128 * g:128 * (g + 1)].astype(F32)

        def u_relayout(j, c):
            for g in range(4):
                ev = ubuf[pl.ds(g * L + 16 * j, 8, stride=2), :]
                od = ubuf[pl.ds(g * L + 16 * j + 1, 8, stride=2), :]
                pa[pl.ds((A_RE + 8 * j) * 8 + g, 8, stride=8), :] = ev
                pa[pl.ds((A_IM + 8 * j) * 8 + g, 8, stride=8), :] = od
            return c
        jax.lax.fori_loop(0, 128, u_relayout, 0)

    kscale = 2.0 ** -14

    def seeds(j):
        for qq in range(4):
            np_ = 4 * j + qq
            ar = dt8 * ld(ppar, 0 * 64 + np_)
            ai = dt8 * ld(ppar, 1 * 64 + np_)
            dbr = dt8 * ld(ppar, 2 * 64 + np_)
            dbi = dt8 * ld(ppar, 3 * 64 + np_)
            cr = ld(ppar, 4 * 64 + np_)
            ci = ld(ppar, 5 * 64 + np_)
            st(ps, C_RE + np_, (cr * dbr - ci * dbi) * kscale)
            st(ps, C_IM + np_, (cr * dbi + ci * dbr) * kscale)
            for q0, mult in ((0, 1.0), (6, 64.0)):
                zr, zi = _cexp(ar * mult, ai * mult)
                for q in range(q0, q0 + 6):
                    st(ps, SEED_RE + q * 64 + np_, zr)
                    st(ps, SEED_IM + q * 64 + np_, zi)
                    if q < q0 + 5:
                        zr, zi = zr * zr - zi * zi, 2.0 * (zr * zi)
    run_vpu('seeds', seeds, 16, 8)

    for s in (3, 2, 1, 0):
        sig = 1 << s
        blocks = [(0, 0), (1, 128)] if s == 0 else [(0, 128)]
        nj1 = 9 if s == 3 else 8
        nit = 16 if s == 0 else 8

        def tables(j, s=s, blocks=blocks, nj1=nj1):
            for qq in range(8):
                np_ = 8 * j + qq
                ev = [None] * 16
                ev[0] = (jnp.ones((8, 128), F32), jnp.zeros((8, 128), F32))
                for j0 in range(1, 16):
                    hb = 1 << (j0.bit_length() - 1)
                    sq = sd(s + hb.bit_length() - 1, np_)
                    ev[j0] = sq if j0 == hb else cmul(*ev[j0 - hb], *sq)
                for j0 in range(16):
                    st(ptab, E_RE + np_ * 16 + j0, ev[j0][0])
                    st(ptab, E_IM + np_ * 16 + j0, ev[j0][1])
                c0 = (ld(ps, C_RE + np_), ld(ps, C_IM + np_))
                for bslot, off in blocks:
                    gv = [None] * nj1
                    gv[0] = c0 if off == 0 else cmul(*c0, *sd(s + 7, np_))
                    for j1 in range(1, nj1):
                        hb = 1 << (j1.bit_length() - 1)
                        gv[j1] = cmul(*gv[j1 - hb], *sd(s + 4 + hb.bit_length() - 1, np_))
                    for j1 in range(nj1):
                        st(ptab, G_RE + (bslot * 8 + j1) * 64 + np_, gv[j1][0])
                        st(ptab, G_IM + (bslot * 8 + j1) * 64 + np_, gv[j1][1])
        run_vpu('tables%d' % s, tables, 8, 8)

        def chunk(j):
            it = j // 4
            ck = j % 4
            acc = jnp.zeros((16, 8, 128), F32)
            for q in range(16):
                np_ = ck * 16 + q
                er = ptab[pl.ds(pl.multiple_of((E_RE + np_ * 16) * 8, 8), 128), :].reshape(16, 8, 128)
                ei = ptab[pl.ds(pl.multiple_of((E_IM + np_ * 16) * 8, 8), 128), :].reshape(16, 8, 128)
                gr = ld(ptab, G_RE + it * 64 + np_)
                gi = ld(ptab, G_IM + it * 64 + np_)
                acc = acc + (gr[None] * er - gi[None] * ei)
            ptab[pl.ds(pl.multiple_of((ACC + j * 16) * 8, 8), 128), :] = acc.reshape(128, 128)
        run_vpu('kgen%d' % s, chunk, nit * 4, 8)

        def scatter(it, s=s, sig=sig):
            acc = ptab[pl.ds(pl.multiple_of((ACC + it * 64) * 8, 8), 128), :]
            for ck in range(1, 4):
                acc = acc + ptab[pl.ds(pl.multiple_of((ACC + it * 64 + ck * 16) * 8, 8), 128), :]
            acc = acc.reshape(16, 8, 128)
            l0 = 16 * it if s == 0 else sig * (128 + 16 * it)
            h0 = l0 // 2
            for j0 in range(16):
                v = acc[j0]
                v = v + swaph(v)
                if sig == 1:
                    box = (0,)
                elif j0 % 2 == 0:
                    box = tuple(range(-(sig // 2), sig // 2 + 1))
                else:
                    box = tuple(range(-(sig // 2) + 1, sig // 2))
                for dlt in box:
                    t_off = sig * j0 + dlt
                    st_k(t_off & 1, h0 + (t_off >> 1), v)
        with jax.named_scope('V_scatter'):
            jax.lax.fori_loop(0, nit, lambda it, c, scatter=scatter: (scatter(it), c)[1], 0)

        if s == 3:
            def body2048(np_, acc):
                return acc + ld(ptab, G_RE + 8 * 64 + np_)
            acc = jax.lax.fori_loop(0, 64, body2048, jnp.zeros((8, 128), F32), unroll=8)
            v = acc + swaph(acc)
            for t in range(2044, 2048):
                st_k(t & 1, t >> 1, v)

    for br in range(2):
        def fwd1(n2, br=br):
            xs = [(ld(pa, A_RE + 32 * n1 + n2), ld(pa, A_IM + 32 * n1 + n2)) for n1 in range(32)]
            if br == 1:
                xs2 = []
                for n1 in range(32):
                    wr, wi = tw(2 * (32 * n1 + n2))
                    xr, xi = xs[n1]
                    xs2.append((xr * wr - xi * wi, xr * wi + xi * wr))
                xs = xs2
            ys = _dft(xs, -1)
            for k1 in range(32):
                yr, yi = ys[k1]
                if k1 > 0:
                    wr, wi = tw(4 * k1 * n2)
                    yr, yi = yr * wr - yi * wi, yr * wi + yi * wr
                st(pb, B_RE + br * 1024 + k1 * 32 + n2, yr)
                st(pb, B_IM + br * 1024 + k1 * 32 + n2, yi)
        run_vpu('fwd1_%d' % br, fwd1, 32, 8)

    def fwd2(gk):
        br = gk // 32
        k1 = gk % 32
        xs = [(ld(pb, B_RE + gk * 32 + n2), ld(pb, B_IM + gk * 32 + n2)) for n2 in range(32)]
        ys = _dft(xs, -1)
        for k2 in range(32):
            k = 2 * (k1 + 32 * k2) + br
            st(pa, A_RE + k, ys[k2][0])
            st(pa, A_IM + k, ys[k2][1])
    run_vpu('fwd2', fwd2, 64, 8)

    M = 2048

    def post(j):
        for qq in range(8):
            k2 = jnp.minimum(8 * j + qq, 512)
            for par in range(2):
                k = 2 * k2 + par
                kb = (M - k) & (M - 1)
                ar, ai = ld(pa, A_RE + k), ld(pa, A_IM + k)
                br_, bi_ = ld(pa, A_RE + kb), ld(pa, A_IM + kb)
                wr, wi = tw(k)
                er = ar + br_
                ei = ai - bi_
                dr = ar - br_
                di = ai + bi_
                tr = wr * di + wi * dr
                ti = wi * di - wr * dr
                x1r, x1i = er + tr, ei + ti
                x2r, x2i = er - tr, ti - ei
                r1r, r1i = swaph(x1r), swaph(x1i)
                r2r, r2i = swaph(x2r), swaph(x2i)
                y1r = x1r * r1r - x1i * r1i
                y1i = x1r * r1i + x1i * r1r
                y2r = x2r * r2r - x2i * r2i
                y2i = x2r * r2i + x2i * r2r
                yer = y1r + y2r
                yei = y1i - y2i
                qr = y1r - y2r
                qi = y1i + y2i
                yor = qr * wr + qi * wi
                yoi = qi * wr - qr * wi
                z1r = yer - yoi
                z1i = yei + yor
                z2r = yer + yoi
                z2i = yor - yei
                q1 = k2
                q2 = (1024 - k2) if par == 0 else (1023 - k2)
                lo = 4 * par
                for q, vr, vi in ((q1, z1r, z1i), (q2, z2r, z2i)):
                    qq_ = jnp.where(q > 1023, 0, q) if par == 0 else q
                    pb[pl.ds(pl.multiple_of((B_RE + qq_) * 8, 8) + lo, 4), :] = vr[lo:lo + 4]
                    pb[pl.ds(pl.multiple_of((B_IM + qq_) * 8, 8) + lo, 4), :] = vi[lo:lo + 4]
    run_vpu('post', post, 66, 11)

    def inv1(n2):
        xs = [(ld(pb, B_RE + 32 * n1 + n2), ld(pb, B_IM + 32 * n1 + n2)) for n1 in range(32)]
        ys = _dft(xs, +1)
        for k1 in range(32):
            yr, yi = ys[k1]
            if k1 > 0:
                wr, wi = tw(4 * k1 * n2)
                wi = -wi
                yr, yi = yr * wr - yi * wi, yr * wi + yi * wr
            st(pa, A_RE + k1 * 32 + n2, yr)
            st(pa, A_IM + k1 * 32 + n2, yi)
    run_vpu('inv1', inv1, 32, 8)

    def inv2(k1):
        xs = [(ld(pa, A_RE + k1 * 32 + n2), ld(pa, A_IM + k1 * 32 + n2)) for n2 in range(32)]
        ys = _dft(xs, +1)
        for k2 in range(32):
            st(pb, B_RE + k1 + 32 * k2, ys[k2][0])
            st(pb, B_IM + k1 + 32 * k2, ys[k2][1])
    run_vpu('inv2', inv2, 32, 8)

    def comb(j):
        for qq in range(32):
            m = 32 * j + qq
            vr, vi = ld(pb, B_RE + m), ld(pb, B_IM + m)
            wr, wi = tw(2 * m)
            wi = -wi
            rr, ri = swaph(vr), swaph(vi)
            st(pa, A_RE + m, vr + (rr * wr - ri * wi))
            st(pa, A_IM + m, vi + (rr * wi + ri * wr))
    run_vpu('comb', comb, 32, 16)

    def y_out(jj):
        for qq in range(4):
            j = 4 * jj + qq
            for g in range(4):
                ev = pa[pl.ds((A_RE + 8 * j) * 8 + g, 8, stride=8), :]
                od = pa[pl.ds((A_IM + 8 * j) * 8 + g, 8, stride=8), :]
                ybuf[pl.ds(g * L + 16 * j, 8, stride=2), :] = ev
                ybuf[pl.ds(g * L + 16 * j + 1, 8, stride=2), :] = od
        r0 = pl.multiple_of(64 * jj, 64)
        for g in range(4):
            dsk = dsk_ref[:, 128 * g:128 * (g + 1)].astype(F32)
            yb = ybuf[pl.ds(g * L + r0, 64), :].astype(BF16).astype(F32)
            sk = (ubuf[pl.ds(g * L + r0, 64), :] * dsk).astype(BF16).astype(F32)
            o_ref[pl.ds(r0, 64), 512 + 128 * g:512 + 128 * (g + 1)] = (yb + sk).astype(BF16)
    run_vpu('yout', y_out, 32, 16)

    flush_mxu()
    with jax.named_scope('M_o'):
        for j in range(S // QRB):
            o_unit(j)


@jax.jit
def pallas_concat_heads__sliding_block__ssm_conv_s4__prompt_kernel(
    A_x: jax.Array,
    A_wqkv: jax.Array,
    A_wo: jax.Array,
    B_u: jax.Array,
    B_A_re: jax.Array,
    B_A_im: jax.Array,
    B_B_re: jax.Array,
    B_B_im: jax.Array,
    B_C_re: jax.Array,
    B_C_im: jax.Array,
    B_log_dt: jax.Array,
    B_Dskip: jax.Array,
):
    vm = pl.BlockSpec(memory_space=pltpu.VMEM)
    out = pl.pallas_call(
        _kernel,
        out_shape=jax.ShapeDtypeStruct((S, 2 * D), BF16),
        in_specs=[pl.BlockSpec(memory_space=pltpu.SMEM)] + [vm] * 12,
        out_specs=vm,
        scratch_shapes=[
            pltpu.VMEM((S, D), BF16),
            pltpu.VMEM((32 * NKB * 128, 128), BF16),
            pltpu.VMEM((32 * 32, 256 + S), BF16),
            pltpu.VMEM((D, S), BF16),
            pltpu.VMEM((4096 * 8, 128), F32),
            pltpu.VMEM((4096 * 8, 128), F32),
            pltpu.VMEM((NSEED * 8, 128), F32),
            pltpu.VMEM((NTAB * 8, 128), F32),
            pltpu.VMEM((384 * 8, 128), F32),
            pltpu.VMEM((4 * L, 128), F32),
            pltpu.VMEM((4 * L, 128), F32),
        ],
        compiler_params=pltpu.CompilerParams(vmem_limit_bytes=120 * 1024 * 1024),
    )(jnp.asarray(_tw_table()), A_x.reshape(S, D), A_wqkv, A_wo, B_u.reshape(L, D),
      B_A_re, B_A_im, B_B_re, B_B_im, B_C_re, B_C_im, B_log_dt.reshape(4, 128), B_Dskip.reshape(1, D))
    return out.reshape(1, S, 2 * D)
```

```python
import math

import numpy as np
import jax
import jax.numpy as jnp
import jax.experimental.pallas as pl
import jax.experimental.pallas.tpu as pltpu

F32 = jnp.float32
BF16 = jnp.bfloat16

S = 2048
D = 512
L = 2048
NEG = -1e30
NKB = 18
QRB = 256
UPI = 4


def _exp_acc(x):
    x = jnp.maximum(x, -87.0)
    k = jnp.floor(x * 1.44269504088896341 + 0.5)
    r = x - k * 0.693359375
    r = r - k * (-2.12194440e-4)
    p = 1.9875691500e-4
    for cf in (1.3981999507e-3, 8.3334519073e-3, 4.1665795894e-2, 1.6666665459e-1, 5.0000001201e-1):
        p = p * r + cf
    p = p * (r * r) + r + 1.0
    ki = k.astype(jnp.int32)
    sc = jax.lax.bitcast_convert_type((ki + 127) << 23, F32)
    return p * sc


def _sincos_acc(t):
    k = jnp.floor(t * 0.636619772367581343 + 0.5)
    r = t - k * 1.5703125
    r = r - k * 4.837512969970703125e-4
    r = r - k * 7.54978995489188216e-8
    r2 = r * r
    s = ((-1.9515295891e-4 * r2 + 8.3321608736e-3) * r2 + (-1.6666654611e-1)) * (r2 * r) + r
    c = ((2.443315711809948e-5 * r2 + (-1.388731625493765e-3)) * r2 + 4.166664568298827e-2) * (r2 * r2) \
        - 0.5 * r2 + 1.0
    q = k.astype(jnp.int32) & 3
    swap = (q & 1) == 1
    sn = jnp.where(swap, c, s)
    cs = jnp.where(swap, s, c)
    sn = jnp.where(q >= 2, -sn, sn)
    cs = jnp.where((q == 1) | (q == 2), -cs, cs)
    return sn, cs


def _cexp(xr, xi):
    e = _exp_acc(xr)
    s, c = _sincos_acc(xi)
    return e * c, e * s


def _cmul_const(xr, xi, wr, wi):
    eps = 1e-12
    if abs(wi) < eps:
        if abs(wr - 1) < eps:
            return xr, xi
        if abs(wr + 1) < eps:
            return -xr, -xi
    if abs(wr) < eps:
        if abs(wi - 1) < eps:
            return -xi, xr
        if abs(wi + 1) < eps:
            return xi, -xr
    if abs(abs(wr) - abs(wi)) < eps:
        s = abs(wr)
        a = 1.0 if wr > 0 else -1.0
        b = 1.0 if wi > 0 else -1.0
        if a * b > 0:
            return (xr - xi) * (a * s), (xr + xi) * (a * s)
        return (xr + xi) * (a * s), (xr - xi) * (-a * s)
    return xr * wr - xi * wi, xr * wi + xi * wr


def _dft(xs, sign):
    n = len(xs)
    if n == 1:
        return xs
    ev = _dft(xs[0::2], sign)
    od = _dft(xs[1::2], sign)
    out = [None] * n
    for k in range(n // 2):
        ang = sign * 2 * math.pi * k / n
        tr, ti = _cmul_const(od[k][0], od[k][1], math.cos(ang), math.sin(ang))
        er, ei = ev[k]
        out[k] = (er + tr, ei + ti)
        out[k + n // 2] = (er - tr, ei - ti)
    return out


A_RE, A_IM = 0, 2048
B_RE, B_IM = 0, 2048
SEED_RE = 0
SEED_IM = SEED_RE + 768
C_RE = SEED_RE + 1536
C_IM = C_RE + 64
NSEED = C_RE + 128
E_RE, E_IM = 0, 1024
G_RE, G_IM = 2048, 2048 + 1088
ACC = G_IM + 1088
NTAB = ACC + 1024
TWN = 4096


def _tw_table():
    e = np.arange(TWN)
    return np.stack([np.cos(2 * np.pi * e / TWN), np.sin(2 * np.pi * e / TWN)]).astype(np.float32)


def _kernel(tw_ref, x_hbm, wqkv_hbm, wo_hbm, u_hbm, are_ref, aim_ref, bre_ref, bim_ref, cre_ref, cim_ref,
            ldt_ref, dsk_ref, o_hbm, qs, km, vtx, ob, pa, pb, ps, ptab, ppar, ubuf, ybuf,
            x_ref, wqkv_ref, wo_ref, u_ref, o_ref, sem_in, sem_out):
    cp_x = pltpu.make_async_copy(x_hbm, x_ref, sem_in.at[0])
    cp_w = pltpu.make_async_copy(wqkv_hbm, wqkv_ref, sem_in.at[1])
    cp_u = pltpu.make_async_copy(u_hbm, u_ref, sem_in.at[2])
    cp_wo = pltpu.make_async_copy(wo_hbm, wo_ref, sem_in.at[3])
    cp_x.start()
    cp_w.start()
    lane = jax.lax.broadcasted_iota(jnp.int32, (128, 128), 1)
    row = jax.lax.broadcasted_iota(jnp.int32, (128, 128), 0)
    tri = row <= lane

    def qkv_phase():
        RB = 512
        for r0 in range(0, S, RB):
            xb = x_ref[r0:r0 + RB, :]
            q = jnp.dot(xb, wqkv_ref[:, 0:512], preferred_element_type=F32).astype(BF16)
            qs[r0:r0 + RB, :] = q * jnp.asarray(0.25, BF16)
            k = jnp.dot(xb, wqkv_ref[:, 512:1024], preferred_element_type=F32).astype(BF16)
            for g in range(4):
                for bb in range(RB // 128):
                    kb = k[128 * bb:128 * (bb + 1), 128 * g:128 * (g + 1)]
                    jb = (r0 // 128) + bb + 2
                    for hh in range(8):
                        msk = (lane >= 16 * hh) & (lane < 16 * (hh + 1))
                        km[pl.ds(((g * NKB + jb) * 8 + hh) * 128, 128), :] = jnp.where(msk, kb, jnp.zeros_like(kb))
            v_t = jax.lax.dot_general(wqkv_ref[:, 1024:1536], xb, (((0,), (1,)), ((), ())),
                                      preferred_element_type=F32).astype(BF16)
            for h in range(32):
                vtx[h * 32:h * 32 + 16, 256 + r0:256 + r0 + RB] = v_t[16 * h:16 * (h + 1)]

    def decode(a):
        lo = a < 8
        r = a - 8
        g = jnp.where(lo, a // 2, r // 14)
        i = jnp.where(lo, a % 2, 2 + r % 14)
        return g, i

    def item8(a, masked):
        g, i = decode(a)
        q0 = pl.multiple_of(i * 128, 128)
        g0 = pl.multiple_of(g * 128, 128)
        qi = qs[pl.ds(q0, 128), pl.ds(g0, 128)]
        kw = km[pl.ds(pl.multiple_of((g * NKB + i) * 1024, 1024), 3072), :]
        st_all = jax.lax.dot_general(kw, qi, (((1,), (1,)), ((), ())), preferred_element_type=F32)
        for hh in range(8):
            s0 = st_all[(0 + hh) * 128:(0 + hh) * 128 + 128]
            s1 = st_all[(8 + hh) * 128:(8 + hh) * 128 + 128]
            s2 = st_all[(16 + hh) * 128:(16 + hh) * 128 + 128]
            if masked:
                s0 = jnp.where(i >= 2, s0, NEG)
                s1 = jnp.where(i >= 1, s1, NEG)
            sm = jnp.where(tri, s2, s0)
            m = jnp.maximum(jnp.max(sm, axis=0, keepdims=True), jnp.max(s1, axis=0, keepdims=True))
            pm = jnp.exp(sm - m)
            p1 = jnp.exp(s1 - m)
            pt = jnp.concatenate([jnp.where(tri, 0.0, pm), p1, jnp.where(tri, pm, 0.0)], axis=0).astype(BF16)
            h = g * 8 + hh
            vtw = vtx[pl.ds(pl.multiple_of(h * 32, 32), 32), pl.ds(q0, 384)]
            ot = jnp.dot(vtw, pt, preferred_element_type=F32)
            ob[pl.ds(pl.multiple_of(h * 16, 16), 16), pl.ds(q0, 128)] = (ot[0:16] / ot[16:17]).astype(BF16)

    def a_unit_m(a):
        item8(a, True)

    def a_unit_f(a):
        item8(a, False)

    def out_a(j):
        return pltpu.make_async_copy(o_ref.at[pl.ds(j * QRB, QRB), pl.ds(0, 512)],
                                     o_hbm.at[pl.ds(j * QRB, QRB), pl.ds(0, 512)], sem_out.at[1 + j])

    out_b = pltpu.make_async_copy(o_ref.at[:, pl.ds(512, 512)], o_hbm.at[:, pl.ds(512, 512)], sem_out.at[0])

    def o_unit(j):
        r0 = pl.multiple_of(j * QRB, QRB)
        o = jax.lax.dot_general(ob[:, pl.ds(r0, QRB)], wo_ref[...], (((0,), (0,)), ((), ())),
                                preferred_element_type=F32)
        o_ref[pl.ds(r0, QRB), 0:512] = o.astype(BF16)
        out_a(j).start()

    mxu_fns = {'am': a_unit_m, 'af': a_unit_f}
    mxu_q = [['am', 0, 8], ['af', 8, 56]]

    def a_prologue():
        stage_a(0)
        stage_b(0, True)
        stage_a(1)

    def a_epilogue():
        stage_c(510)
        stage_b(511, False)
        stage_c(511)

    def next_mxu():
        while mxu_q and mxu_q[0][0] in ('pro', 'epi'):
            kind = mxu_q.pop(0)[0]
            a_prologue() if kind == 'pro' else a_epilogue()
        return mxu_q[0] if mxu_q else None

    carry_units = []

    def run_vpu(name, fn, n, upi_a):
        done = 0
        while done < n:
            seg = next_mxu()
            if seg is None:
                cnt = n - done
                base_v = done
                with jax.named_scope('V_' + name):
                    jax.lax.fori_loop(0, cnt, lambda j, c, base_v=base_v: (fn(base_v + j), c)[1], 0)
                done += cnt
                continue
            kind, start, left = seg
            upi = upi_a
            rem = n - done
            if rem < upi:
                base_v = done
                with jax.named_scope('V_' + name):
                    jax.lax.fori_loop(0, rem, lambda j, c, base_v=base_v: (fn(base_v + j), c)[1], 0)
                done += rem
                continue
            cnt = min(rem // upi, left)
            base_v, base_m, mf = done, start, mxu_fns[kind]

            def body(j, c, base_v=base_v, base_m=base_m, mf=mf, upi=upi):
                mf(base_m + j)
                for q in range(upi):
                    fn(base_v + j * upi + q)
                return c
            with jax.named_scope('F_' + name + '_' + kind):
                jax.lax.fori_loop(0, cnt, body, 0)
            seg[1] += cnt
            seg[2] -= cnt
            if seg[2] == 0:
                mxu_q.pop(0)
            done += cnt * upi

    def flush_mxu():
        while True:
            seg = next_mxu()
            if seg is None:
                break
            kind, start, left = seg
            mf = mxu_fns[kind]
            with jax.named_scope('M_' + kind):
                jax.lax.fori_loop(0, left, lambda j, c, start=start, mf=mf: (mf(start + j), c)[1], 0)
            mxu_q.pop(0)

    def ld(ref, i):
        return ref[pl.ds(pl.multiple_of(i * 8, 8), 8), :]

    def st(ref, i, v):
        ref[pl.ds(pl.multiple_of(i * 8, 8), 8), :] = v

    def swaph(v):
        return pltpu.roll(v, 4, 0)

    def cmul(ar, ai, br, bi):
        return ar * br - ai * bi, ar * bi + ai * br

    def sd(q, np_):
        return ld(ps, SEED_RE + q * 64 + np_), ld(ps, SEED_IM + q * 64 + np_)

    def st_k(t_par, m, v):
        base = A_IM if t_par else A_RE
        pa[pl.ds(pl.multiple_of((base + m) * 8, 8) + 4, 4), :] = v[4:8]

    def tw(e):
        return tw_ref[0, e], -tw_ref[1, e]

    zk = jnp.zeros((2048, 128), BF16)
    for g in range(4):
        km[pl.ds((g * NKB) * 1024, 2048), :] = zk
    r32 = jax.lax.broadcasted_iota(jnp.int32, (16, 256 + S), 0)
    ones_blk = jnp.where(r32 == 0, 1.0, 0.0).astype(BF16)
    for h in range(32):
        vtx[pl.ds(h * 32 + 16, 16), :] = ones_blk
        vtx[pl.ds(h * 32, 16), 0:256] = jnp.zeros((16, 256), BF16)

    with jax.named_scope('B0'):
        for a_i, ref in enumerate((are_ref, aim_ref, bre_ref, bim_ref, cre_ref, cim_ref)):
            for g in range(4):
                blk = ref[128 * g:128 * (g + 1), :].astype(F32)
                ppar[pl.ds((a_i * 64) * 8 + g, 128, stride=4), :] = blk.T
        dt4 = _exp_acc(ldt_ref[...].astype(F32)).astype(BF16).astype(F32)
        dt8 = jnp.concatenate([dt4, dt4], axis=0)
    cp_x.wait()
    cp_w.wait()
    cp_u.start()
    cp_wo.start()
    with jax.named_scope('QKV'):
        qkv_phase()
    cp_u.wait()
    with jax.named_scope('B0u'):
        for g in range(4):
            for r0 in range(0, L, 256):
                ubuf[g * L + r0:g * L + r0 + 256, :] = u_ref[r0:r0 + 256, 128 * g:128 * (g + 1)].astype(F32)

        def u_relayout(j, c):
            for g in range(4):
                ev = ubuf[pl.ds(g * L + 16 * j, 8, stride=2), :]
                od = ubuf[pl.ds(g * L + 16 * j + 1, 8, stride=2), :]
                pa[pl.ds((A_RE + 8 * j) * 8 + g, 8, stride=8), :] = ev
                pa[pl.ds((A_IM + 8 * j) * 8 + g, 8, stride=8), :] = od
            return c
        jax.lax.fori_loop(0, 128, u_relayout, 0)

    kscale = 2.0 ** -14

    def seeds(j):
        for qq in range(4):
            np_ = 4 * j + qq
            ar = dt8 * ld(ppar, 0 * 64 + np_)
            ai = dt8 * ld(ppar, 1 * 64 + np_)
            dbr = dt8 * ld(ppar, 2 * 64 + np_)
            dbi = dt8 * ld(ppar, 3 * 64 + np_)
            cr = ld(ppar, 4 * 64 + np_)
            ci = ld(ppar, 5 * 64 + np_)
            st(ps, C_RE + np_, (cr * dbr - ci * dbi) * kscale)
            st(ps, C_IM + np_, (cr * dbi + ci * dbr) * kscale)
            for q0, mult in ((0, 1.0), (6, 64.0)):
                zr, zi = _cexp(ar * mult, ai * mult)
                for q in range(q0, q0 + 6):
                    st(ps, SEED_RE + q * 64 + np_, zr)
                    st(ps, SEED_IM + q * 64 + np_, zi)
                    if q < q0 + 5:
                        zr, zi = zr * zr - zi * zi, 2.0 * (zr * zi)
    run_vpu('seeds', seeds, 16, 8)

    for s in (3, 2, 1, 0):
        sig = 1 << s
        blocks = [(0, 0), (1, 128)] if s == 0 else [(0, 128)]
        nj1 = 9 if s == 3 else 8
        nit = 16 if s == 0 else 8

        def tables(j, s=s, blocks=blocks, nj1=nj1):
            for qq in range(8):
                np_ = 8 * j + qq
                ev = [None] * 16
                ev[0] = (jnp.ones((8, 128), F32), jnp.zeros((8, 128), F32))
                for j0 in range(1, 16):
                    hb = 1 << (j0.bit_length() - 1)
                    sq = sd(s + hb.bit_length() - 1, np_)
                    ev[j0] = sq if j0 == hb else cmul(*ev[j0 - hb], *sq)
                for j0 in range(16):
                    st(ptab, E_RE + np_ * 16 + j0, ev[j0][0])
                    st(ptab, E_IM + np_ * 16 + j0, ev[j0][1])
                c0 = (ld(ps, C_RE + np_), ld(ps, C_IM + np_))
                for bslot, off in blocks:
                    gv = [None] * nj1
                    gv[0] = c0 if off == 0 else cmul(*c0, *sd(s + 7, np_))
                    for j1 in range(1, nj1):
                        hb = 1 << (j1.bit_length() - 1)
                        gv[j1] = cmul(*gv[j1 - hb], *sd(s + 4 + hb.bit_length() - 1, np_))
                    for j1 in range(nj1):
                        st(ptab, G_RE + (bslot * 8 + j1) * 64 + np_, gv[j1][0])
                        st(ptab, G_IM + (bslot * 8 + j1) * 64 + np_, gv[j1][1])
        run_vpu('tables%d' % s, tables, 8, 8)

        def chunk(j):
            it = j // 4
            ck = j % 4
            acc = jnp.zeros((16, 8, 128), F32)
            for q in range(16):
                np_ = ck * 16 + q
                er = ptab[pl.ds(pl.multiple_of((E_RE + np_ * 16) * 8, 8), 128), :].reshape(16, 8, 128)
                ei = ptab[pl.ds(pl.multiple_of((E_IM + np_ * 16) * 8, 8), 128), :].reshape(16, 8, 128)
                gr = ld(ptab, G_RE + it * 64 + np_)
                gi = ld(ptab, G_IM + it * 64 + np_)
                acc = acc + (gr[None] * er - gi[None] * ei)
            ptab[pl.ds(pl.multiple_of((ACC + j * 16) * 8, 8), 128), :] = acc.reshape(128, 128)
        run_vpu('kgen%d' % s, chunk, nit * 4, 8)

        def scatter(it, s=s, sig=sig):
            acc = ptab[pl.ds(pl.multiple_of((ACC + it * 64) * 8, 8), 128), :]
            for ck in range(1, 4):
                acc = acc + ptab[pl.ds(pl.multiple_of((ACC + it * 64 + ck * 16) * 8, 8), 128), :]
            acc = acc.reshape(16, 8, 128)
            l0 = 16 * it if s == 0 else sig * (128 + 16 * it)
            h0 = l0 // 2
            for j0 in range(16):
                v = acc[j0]
                v = v + swaph(v)
                if sig == 1:
                    box = (0,)
                elif j0 % 2 == 0:
                    box = tuple(range(-(sig // 2), sig // 2 + 1))
                else:
                    box = tuple(range(-(sig // 2) + 1, sig // 2))
                for dlt in box:
                    t_off = sig * j0 + dlt
                    st_k(t_off & 1, h0 + (t_off >> 1), v)
        with jax.named_scope('V_scatter'):
            jax.lax.fori_loop(0, nit, lambda it, c, scatter=scatter: (scatter(it), c)[1], 0)

        if s == 3:
            def body2048(np_, acc):
                return acc + ld(ptab, G_RE + 8 * 64 + np_)
            acc = jax.lax.fori_loop(0, 64, body2048, jnp.zeros((8, 128), F32), unroll=8)
            v = acc + swaph(acc)
            for t in range(2044, 2048):
                st_k(t & 1, t >> 1, v)

    for br in range(2):
        def fwd1(n2, br=br):
            xs = [(ld(pa, A_RE + 32 * n1 + n2), ld(pa, A_IM + 32 * n1 + n2)) for n1 in range(32)]
            if br == 1:
                xs2 = []
                for n1 in range(32):
                    wr, wi = tw(2 * (32 * n1 + n2))
                    xr, xi = xs[n1]
                    xs2.append((xr * wr - xi * wi, xr * wi + xi * wr))
                xs = xs2
            ys = _dft(xs, -1)
            for k1 in range(32):
                yr, yi = ys[k1]
                if k1 > 0:
                    wr, wi = tw(4 * k1 * n2)
                    yr, yi = yr * wr - yi * wi, yr * wi + yi * wr
                st(pb, B_RE + br * 1024 + k1 * 32 + n2, yr)
                st(pb, B_IM + br * 1024 + k1 * 32 + n2, yi)
        run_vpu('fwd1_%d' % br, fwd1, 32, 8)

    def fwd2(gk):
        br = gk // 32
        k1 = gk % 32
        xs = [(ld(pb, B_RE + gk * 32 + n2), ld(pb, B_IM + gk * 32 + n2)) for n2 in range(32)]
        ys = _dft(xs, -1)
        for k2 in range(32):
            k = 2 * (k1 + 32 * k2) + br
            st(pa, A_RE + k, ys[k2][0])
            st(pa, A_IM + k, ys[k2][1])
    run_vpu('fwd2', fwd2, 64, 8)

    M = 2048

    def post(j):
        for qq in range(8):
            k2 = jnp.minimum(8 * j + qq, 512)
            for par in range(2):
                k = 2 * k2 + par
                kb = (M - k) & (M - 1)
                ar, ai = ld(pa, A_RE + k), ld(pa, A_IM + k)
                br_, bi_ = ld(pa, A_RE + kb), ld(pa, A_IM + kb)
                wr, wi = tw(k)
                er = ar + br_
                ei = ai - bi_
                dr = ar - br_
                di = ai + bi_
                tr = wr * di + wi * dr
                ti = wi * di - wr * dr
                x1r, x1i = er + tr, ei + ti
                x2r, x2i = er - tr, ti - ei
                r1r, r1i = swaph(x1r), swaph(x1i)
                r2r, r2i = swaph(x2r), swaph(x2i)
                y1r = x1r * r1r - x1i * r1i
                y1i = x1r * r1i + x1i * r1r
                y2r = x2r * r2r - x2i * r2i
                y2i = x2r * r2i + x2i * r2r
                yer = y1r + y2r
                yei = y1i - y2i
                qr = y1r - y2r
                qi = y1i + y2i
                yor = qr * wr + qi * wi
                yoi = qi * wr - qr * wi
                z1r = yer - yoi
                z1i = yei + yor
                z2r = yer + yoi
                z2i = yor - yei
                q1 = k2
                q2 = (1024 - k2) if par == 0 else (1023 - k2)
                lo = 4 * par
                for q, vr, vi in ((q1, z1r, z1i), (q2, z2r, z2i)):
                    qq_ = jnp.where(q > 1023, 0, q) if par == 0 else q
                    pb[pl.ds(pl.multiple_of((B_RE + qq_) * 8, 8) + lo, 4), :] = vr[lo:lo + 4]
                    pb[pl.ds(pl.multiple_of((B_IM + qq_) * 8, 8) + lo, 4), :] = vi[lo:lo + 4]
    run_vpu('post', post, 72, 9)

    def inv1(n2):
        xs = [(ld(pb, B_RE + 32 * n1 + n2), ld(pb, B_IM + 32 * n1 + n2)) for n1 in range(32)]
        ys = _dft(xs, +1)
        for k1 in range(32):
            yr, yi = ys[k1]
            if k1 > 0:
                wr, wi = tw(4 * k1 * n2)
                wi = -wi
                yr, yi = yr * wr - yi * wi, yr * wi + yi * wr
            st(pa, A_RE + k1 * 32 + n2, yr)
            st(pa, A_IM + k1 * 32 + n2, yi)
    run_vpu('inv1', inv1, 32, 8)

    def inv2(k1):
        xs = [(ld(pa, A_RE + k1 * 32 + n2), ld(pa, A_IM + k1 * 32 + n2)) for n2 in range(32)]
        ys = _dft(xs, +1)
        for k2 in range(32):
            st(pb, B_RE + k1 + 32 * k2, ys[k2][0])
            st(pb, B_IM + k1 + 32 * k2, ys[k2][1])
    run_vpu('inv2', inv2, 32, 8)

    def comb(j):
        for qq in range(32):
            m = 32 * j + qq
            vr, vi = ld(pb, B_RE + m), ld(pb, B_IM + m)
            wr, wi = tw(2 * m)
            wi = -wi
            rr, ri = swaph(vr), swaph(vi)
            st(pa, A_RE + m, vr + (rr * wr - ri * wi))
            st(pa, A_IM + m, vi + (rr * wi + ri * wr))
    run_vpu('comb', comb, 32, 8)

    def y_out(jj):
        for qq in range(4):
            j = 4 * jj + qq
            for g in range(4):
                ev = pa[pl.ds((A_RE + 8 * j) * 8 + g, 8, stride=8), :]
                od = pa[pl.ds((A_IM + 8 * j) * 8 + g, 8, stride=8), :]
                ybuf[pl.ds(g * L + 16 * j, 8, stride=2), :] = ev
                ybuf[pl.ds(g * L + 16 * j + 1, 8, stride=2), :] = od
        r0 = pl.multiple_of(64 * jj, 64)
        for g in range(4):
            dsk = dsk_ref[:, 128 * g:128 * (g + 1)].astype(F32)
            yb = ybuf[pl.ds(g * L + r0, 64), :].astype(BF16).astype(F32)
            sk = (ubuf[pl.ds(g * L + r0, 64), :] * dsk).astype(BF16).astype(F32)
            o_ref[pl.ds(r0, 64), 512 + 128 * g:512 + 128 * (g + 1)] = (yb + sk).astype(BF16)
    run_vpu('yout', y_out, 32, 16)
    out_b.start()

    flush_mxu()
    cp_wo.wait()
    with jax.named_scope('M_o'):
        for j in range(S // QRB):
            o_unit(j)
    out_b.wait()
    for j in range(S // QRB):
        out_a(j).wait()


@jax.jit
def pallas_concat_heads__sliding_block__ssm_conv_s4__prompt_kernel(
    A_x: jax.Array,
    A_wqkv: jax.Array,
    A_wo: jax.Array,
    B_u: jax.Array,
    B_A_re: jax.Array,
    B_A_im: jax.Array,
    B_B_re: jax.Array,
    B_B_im: jax.Array,
    B_C_re: jax.Array,
    B_C_im: jax.Array,
    B_log_dt: jax.Array,
    B_Dskip: jax.Array,
):
    vm = pl.BlockSpec(memory_space=pltpu.VMEM)
    hbm = pl.BlockSpec(memory_space=pl.ANY)
    out = pl.pallas_call(
        _kernel,
        out_shape=jax.ShapeDtypeStruct((S, 2 * D), BF16),
        in_specs=[pl.BlockSpec(memory_space=pltpu.SMEM)] + [hbm] * 4 + [vm] * 8,
        out_specs=hbm,
        scratch_shapes=[
            pltpu.VMEM((S, D), BF16),
            pltpu.VMEM((32 * NKB * 128, 128), BF16),
            pltpu.VMEM((32 * 32, 256 + S), BF16),
            pltpu.VMEM((D, S), BF16),
            pltpu.VMEM((4096 * 8, 128), F32),
            pltpu.VMEM((4096 * 8, 128), F32),
            pltpu.VMEM((NSEED * 8, 128), F32),
            pltpu.VMEM((NTAB * 8, 128), F32),
            pltpu.VMEM((384 * 8, 128), F32),
            pltpu.VMEM((4 * L, 128), F32),
            pltpu.VMEM((4 * L, 128), F32),
            pltpu.VMEM((S, D), BF16),
            pltpu.VMEM((D, 3 * D), BF16),
            pltpu.VMEM((D, D), BF16),
            pltpu.VMEM((L, D), BF16),
            pltpu.VMEM((S, 2 * D), BF16),
            pltpu.SemaphoreType.DMA((4,)),
            pltpu.SemaphoreType.DMA((1 + S // QRB,)),
        ],
        compiler_params=pltpu.CompilerParams(vmem_limit_bytes=120 * 1024 * 1024),
    )(jnp.asarray(_tw_table()), A_x.reshape(S, D), A_wqkv, A_wo, B_u.reshape(L, D),
      B_A_re, B_A_im, B_B_re, B_B_im, B_C_re, B_C_im, B_log_dt.reshape(4, 128), B_Dskip.reshape(1, D))
    return out.reshape(1, S, 2 * D)
```

```python
import math

import numpy as np
import jax
import jax.numpy as jnp
import jax.experimental.pallas as pl
import jax.experimental.pallas.tpu as pltpu

F32 = jnp.float32
BF16 = jnp.bfloat16

S = 2048
D = 512
L = 2048
NEG = -1e30
NKB = 18
QRB = 256
UPI = 4


def _exp_acc(x):
    x = jnp.maximum(x, -87.0)
    k = jnp.floor(x * 1.44269504088896341 + 0.5)
    r = x - k * 0.693359375
    r = r - k * (-2.12194440e-4)
    p = 1.9875691500e-4
    for cf in (1.3981999507e-3, 8.3334519073e-3, 4.1665795894e-2, 1.6666665459e-1, 5.0000001201e-1):
        p = p * r + cf
    p = p * (r * r) + r + 1.0
    ki = k.astype(jnp.int32)
    sc = jax.lax.bitcast_convert_type((ki + 127) << 23, F32)
    return p * sc


def _sincos_acc(t):
    k = jnp.floor(t * 0.636619772367581343 + 0.5)
    r = t - k * 1.5703125
    r = r - k * 4.837512969970703125e-4
    r = r - k * 7.54978995489188216e-8
    r2 = r * r
    s = ((-1.9515295891e-4 * r2 + 8.3321608736e-3) * r2 + (-1.6666654611e-1)) * (r2 * r) + r
    c = ((2.443315711809948e-5 * r2 + (-1.388731625493765e-3)) * r2 + 4.166664568298827e-2) * (r2 * r2) \
        - 0.5 * r2 + 1.0
    q = k.astype(jnp.int32) & 3
    swap = (q & 1) == 1
    sn = jnp.where(swap, c, s)
    cs = jnp.where(swap, s, c)
    sn = jnp.where(q >= 2, -sn, sn)
    cs = jnp.where((q == 1) | (q == 2), -cs, cs)
    return sn, cs


def _cexp(xr, xi):
    e = _exp_acc(xr)
    s, c = _sincos_acc(xi)
    return e * c, e * s


def _cmul_const(xr, xi, wr, wi):
    eps = 1e-12
    if abs(wi) < eps:
        if abs(wr - 1) < eps:
            return xr, xi
        if abs(wr + 1) < eps:
            return -xr, -xi
    if abs(wr) < eps:
        if abs(wi - 1) < eps:
            return -xi, xr
        if abs(wi + 1) < eps:
            return xi, -xr
    if abs(abs(wr) - abs(wi)) < eps:
        s = abs(wr)
        a = 1.0 if wr > 0 else -1.0
        b = 1.0 if wi > 0 else -1.0
        if a * b > 0:
            return (xr - xi) * (a * s), (xr + xi) * (a * s)
        return (xr + xi) * (a * s), (xr - xi) * (-a * s)
    return xr * wr - xi * wi, xr * wi + xi * wr


def _dft(xs, sign):
    n = len(xs)
    if n == 1:
        return xs
    ev = _dft(xs[0::2], sign)
    od = _dft(xs[1::2], sign)
    out = [None] * n
    for k in range(n // 2):
        ang = sign * 2 * math.pi * k / n
        tr, ti = _cmul_const(od[k][0], od[k][1], math.cos(ang), math.sin(ang))
        er, ei = ev[k]
        out[k] = (er + tr, ei + ti)
        out[k + n // 2] = (er - tr, ei - ti)
    return out


A_RE, A_IM = 0, 2048
B_RE, B_IM = 0, 2048
SEED_RE = 0
SEED_IM = SEED_RE + 768
C_RE = SEED_RE + 1536
C_IM = C_RE + 64
NSEED = C_RE + 128
E_RE, E_IM = 0, 1024
G_RE, G_IM = 2048, 2048 + 1088
ACC = G_IM + 1088
NTAB = ACC + 1024
TWN = 4096


def _tw_table():
    e = np.arange(TWN)
    return np.stack([np.cos(2 * np.pi * e / TWN), np.sin(2 * np.pi * e / TWN)]).astype(np.float32)


def _kernel(tw_ref, x_hbm, wqkv_hbm, wo_hbm, u_hbm, are_ref, aim_ref, bre_ref, bim_ref, cre_ref, cim_ref,
            ldt_ref, dsk_ref, o_hbm, qs, km, vtx, ob, pa, pb, ps, ptab, ppar, ubuf, ybuf,
            x_ref, wqkv_ref, wo_ref, u_ref, o_ref, sem_in, sem_out):
    cp_x = pltpu.make_async_copy(x_hbm, x_ref, sem_in.at[0])
    cp_w = pltpu.make_async_copy(wqkv_hbm, wqkv_ref, sem_in.at[1])
    cp_u = pltpu.make_async_copy(u_hbm, u_ref, sem_in.at[2])
    cp_wo = pltpu.make_async_copy(wo_hbm, wo_ref, sem_in.at[3])
    cp_x.start()
    cp_w.start()
    lane = jax.lax.broadcasted_iota(jnp.int32, (128, 128), 1)
    row = jax.lax.broadcasted_iota(jnp.int32, (128, 128), 0)
    tri = row <= lane

    def qkv_phase():
        RB = 512
        for r0 in range(0, S, RB):
            xb = x_ref[r0:r0 + RB, :]
            q = jnp.dot(xb, wqkv_ref[:, 0:512], preferred_element_type=F32).astype(BF16)
            qs[r0:r0 + RB, :] = q * jnp.asarray(0.25, BF16)
            k = jnp.dot(xb, wqkv_ref[:, 512:1024], preferred_element_type=F32).astype(BF16)
            for g in range(4):
                for bb in range(RB // 128):
                    kb = k[128 * bb:128 * (bb + 1), 128 * g:128 * (g + 1)]
                    jb = (r0 // 128) + bb + 2
                    for hh in range(8):
                        msk = (lane >= 16 * hh) & (lane < 16 * (hh + 1))
                        km[pl.ds(((g * NKB + jb) * 8 + hh) * 128, 128), :] = jnp.where(msk, kb, jnp.zeros_like(kb))
            v_t = jax.lax.dot_general(wqkv_ref[:, 1024:1536], xb, (((0,), (1,)), ((), ())),
                                      preferred_element_type=F32).astype(BF16)
            for h in range(32):
                vtx[h * 32:h * 32 + 16, 256 + r0:256 + r0 + RB] = v_t[16 * h:16 * (h + 1)]

    def decode(a):
        lo = a < 8
        r = a - 8
        g = jnp.where(lo, a // 2, r // 14)
        i = jnp.where(lo, a % 2, 2 + r % 14)
        return g, i

    def item8(a, masked):
        g, i = decode(a)
        q0 = pl.multiple_of(i * 128, 128)
        g0 = pl.multiple_of(g * 128, 128)
        qi = qs[pl.ds(q0, 128), pl.ds(g0, 128)]
        kw = km[pl.ds(pl.multiple_of((g * NKB + i) * 1024, 1024), 3072), :]
        st_all = jax.lax.dot_general(kw, qi, (((1,), (1,)), ((), ())), preferred_element_type=F32)
        for hh in range(8):
            s0 = st_all[(0 + hh) * 128:(0 + hh) * 128 + 128]
            s1 = st_all[(8 + hh) * 128:(8 + hh) * 128 + 128]
            s2 = st_all[(16 + hh) * 128:(16 + hh) * 128 + 128]
            if masked:
                s0 = jnp.where(i >= 2, s0, NEG)
                s1 = jnp.where(i >= 1, s1, NEG)
            sm = jnp.where(tri, s2, s0)
            m = jnp.maximum(jnp.max(sm, axis=0, keepdims=True), jnp.max(s1, axis=0, keepdims=True))
            pm = jnp.exp(sm - m)
            p1 = jnp.exp(s1 - m)
            pt = jnp.concatenate([jnp.where(tri, 0.0, pm), p1, jnp.where(tri, pm, 0.0)], axis=0).astype(BF16)
            h = g * 8 + hh
            vtw = vtx[pl.ds(pl.multiple_of(h * 32, 32), 32), pl.ds(q0, 384)]
            ot = jnp.dot(vtw, pt, preferred_element_type=F32)
            ob[pl.ds(pl.multiple_of(h * 16, 16), 16), pl.ds(q0, 128)] = (ot[0:16] / ot[16:17]).astype(BF16)

    def a_unit_m(a):
        item8(a, True)

    def a_unit_f(a):
        item8(a, False)

    def out_a(j):
        return pltpu.make_async_copy(o_ref.at[pl.ds(j * QRB, QRB), pl.ds(0, 512)],
                                     o_hbm.at[pl.ds(j * QRB, QRB), pl.ds(0, 512)], sem_out.at[1 + j])

    out_b = pltpu.make_async_copy(o_ref.at[:, pl.ds(512, 512)], o_hbm.at[:, pl.ds(512, 512)], sem_out.at[0])

    def o_unit(j):
        r0 = pl.multiple_of(j * QRB, QRB)
        o = jax.lax.dot_general(ob[:, pl.ds(r0, QRB)], wo_ref[...], (((0,), (0,)), ((), ())),
                                preferred_element_type=F32)
        o_ref[pl.ds(r0, QRB), 0:512] = o.astype(BF16)
        out_a(j).start()

    mxu_fns = {'am': a_unit_m, 'af': a_unit_f}
    mxu_q = [['am', 0, 8], ['af', 8, 56]]

    def next_mxu():
        return mxu_q[0] if mxu_q else None

    def run_vpu(name, fn, n, upi_a):
        done = 0
        while done < n:
            seg = next_mxu()
            if seg is None:
                cnt = n - done
                base_v = done
                with jax.named_scope('V_' + name):
                    jax.lax.fori_loop(0, cnt, lambda j, c, base_v=base_v: (fn(base_v + j), c)[1], 0)
                done += cnt
                continue
            kind, start, left = seg
            upi = upi_a
            rem = n - done
            if rem < upi:
                base_v = done
                with jax.named_scope('V_' + name):
                    jax.lax.fori_loop(0, rem, lambda j, c, base_v=base_v: (fn(base_v + j), c)[1], 0)
                done += rem
                continue
            cnt = min(rem // upi, left)
            base_v, base_m, mf = done, start, mxu_fns[kind]

            def body(j, c, base_v=base_v, base_m=base_m, mf=mf, upi=upi):
                mf(base_m + j)
                for q in range(upi):
                    fn(base_v + j * upi + q)
                return c
            with jax.named_scope('F_' + name + '_' + kind):
                jax.lax.fori_loop(0, cnt, body, 0)
            seg[1] += cnt
            seg[2] -= cnt
            if seg[2] == 0:
                mxu_q.pop(0)
            done += cnt * upi

    def flush_mxu():
        while True:
            seg = next_mxu()
            if seg is None:
                break
            kind, start, left = seg
            mf = mxu_fns[kind]
            with jax.named_scope('M_' + kind):
                jax.lax.fori_loop(0, left, lambda j, c, start=start, mf=mf: (mf(start + j), c)[1], 0)
            mxu_q.pop(0)

    def ld(ref, i):
        return ref[pl.ds(pl.multiple_of(i * 8, 8), 8), :]

    def st(ref, i, v):
        ref[pl.ds(pl.multiple_of(i * 8, 8), 8), :] = v

    def swaph(v):
        return pltpu.roll(v, 4, 0)

    def cmul(ar, ai, br, bi):
        return ar * br - ai * bi, ar * bi + ai * br

    def sd(q, np_):
        return ld(ps, SEED_RE + q * 64 + np_), ld(ps, SEED_IM + q * 64 + np_)

    def st_k(t_par, m, v):
        base = A_IM if t_par else A_RE
        pa[pl.ds(pl.multiple_of((base + m) * 8, 8) + 4, 4), :] = v[4:8]

    def tw(e):
        return tw_ref[0, e], -tw_ref[1, e]

    zk = jnp.zeros((2048, 128), BF16)
    for g in range(4):
        km[pl.ds((g * NKB) * 1024, 2048), :] = zk
    r32 = jax.lax.broadcasted_iota(jnp.int32, (16, 256 + S), 0)
    ones_blk = jnp.where(r32 == 0, 1.0, 0.0).astype(BF16)
    for h in range(32):
        vtx[pl.ds(h * 32 + 16, 16), :] = ones_blk
        vtx[pl.ds(h * 32, 16), 0:256] = jnp.zeros((16, 256), BF16)

    with jax.named_scope('B0'):
        for a_i, ref in enumerate((are_ref, aim_ref, bre_ref, bim_ref, cre_ref, cim_ref)):
            for g in range(4):
                blk = ref[128 * g:128 * (g + 1), :].astype(F32)
                ppar[pl.ds((a_i * 64) * 8 + g, 128, stride=4), :] = blk.T
        dt4 = _exp_acc(ldt_ref[...].astype(F32)).astype(BF16).astype(F32)
        dt8 = jnp.concatenate([dt4, dt4], axis=0)
    cp_x.wait()
    cp_w.wait()
    cp_u.start()
    cp_wo.start()
    with jax.named_scope('QKV'):
        qkv_phase()
    cp_u.wait()
    with jax.named_scope('B0u'):
        for g in range(4):
            for r0 in range(0, L, 256):
                ubuf[g * L + r0:g * L + r0 + 256, :] = u_ref[r0:r0 + 256, 128 * g:128 * (g + 1)].astype(F32)

        def u_relayout(j, c):
            for g in range(4):
                ev = ubuf[pl.ds(g * L + 16 * j, 8, stride=2), :]
                od = ubuf[pl.ds(g * L + 16 * j + 1, 8, stride=2), :]
                pa[pl.ds((A_RE + 8 * j) * 8 + g, 8, stride=8), :] = ev
                pa[pl.ds((A_IM + 8 * j) * 8 + g, 8, stride=8), :] = od
            return c
        jax.lax.fori_loop(0, 128, u_relayout, 0)

    kscale = 2.0 ** -14

    def seeds(j):
        for qq in range(4):
            np_ = 4 * j + qq
            ar = dt8 * ld(ppar, 0 * 64 + np_)
            ai = dt8 * ld(ppar, 1 * 64 + np_)
            dbr = dt8 * ld(ppar, 2 * 64 + np_)
            dbi = dt8 * ld(ppar, 3 * 64 + np_)
            cr = ld(ppar, 4 * 64 + np_)
            ci = ld(ppar, 5 * 64 + np_)
            st(ps, C_RE + np_, (cr * dbr - ci * dbi) * kscale)
            st(ps, C_IM + np_, (cr * dbi + ci * dbr) * kscale)
            for q0, mult in ((0, 1.0), (6, 64.0)):
                zr, zi = _cexp(ar * mult, ai * mult)
                for q in range(q0, q0 + 6):
                    st(ps, SEED_RE + q * 64 + np_, zr)
                    st(ps, SEED_IM + q * 64 + np_, zi)
                    if q < q0 + 5:
                        zr, zi = zr * zr - zi * zi, 2.0 * (zr * zi)
    run_vpu('seeds', seeds, 16, 8)

    for s in (3, 2, 1, 0):
        sig = 1 << s
        blocks = [(0, 0), (1, 128)] if s == 0 else [(0, 128)]
        nj1 = 9 if s == 3 else 8
        nit = 16 if s == 0 else 8

        def tables(j, s=s, blocks=blocks, nj1=nj1):
            for qq in range(8):
                np_ = 8 * j + qq
                ev = [None] * 16
                ev[0] = (jnp.ones((8, 128), F32), jnp.zeros((8, 128), F32))
                for j0 in range(1, 16):
                    hb = 1 << (j0.bit_length() - 1)
                    sq = sd(s + hb.bit_length() - 1, np_)
                    ev[j0] = sq if j0 == hb else cmul(*ev[j0 - hb], *sq)
                for j0 in range(16):
                    st(ptab, E_RE + np_ * 16 + j0, ev[j0][0])
                    st(ptab, E_IM + np_ * 16 + j0, ev[j0][1])
                c0 = (ld(ps, C_RE + np_), ld(ps, C_IM + np_))
                for bslot, off in blocks:
                    gv = [None] * nj1
                    gv[0] = c0 if off == 0 else cmul(*c0, *sd(s + 7, np_))
                    for j1 in range(1, nj1):
                        hb = 1 << (j1.bit_length() - 1)
                        gv[j1] = cmul(*gv[j1 - hb], *sd(s + 4 + hb.bit_length() - 1, np_))
                    for j1 in range(nj1):
                        st(ptab, G_RE + (bslot * 8 + j1) * 64 + np_, gv[j1][0])
                        st(ptab, G_IM + (bslot * 8 + j1) * 64 + np_, gv[j1][1])
        run_vpu('tables%d' % s, tables, 8, 8)

        def chunk(j):
            it = j // 4
            ck = j % 4
            acc = jnp.zeros((16, 8, 128), F32)
            for q in range(16):
                np_ = ck * 16 + q
                er = ptab[pl.ds(pl.multiple_of((E_RE + np_ * 16) * 8, 8), 128), :].reshape(16, 8, 128)
                ei = ptab[pl.ds(pl.multiple_of((E_IM + np_ * 16) * 8, 8), 128), :].reshape(16, 8, 128)
                gr = ld(ptab, G_RE + it * 64 + np_)
                gi = ld(ptab, G_IM + it * 64 + np_)
                acc = acc + (gr[None] * er - gi[None] * ei)
            ptab[pl.ds(pl.multiple_of((ACC + j * 16) * 8, 8), 128), :] = acc.reshape(128, 128)
        run_vpu('kgen%d' % s, chunk, nit * 4, 8)

        def scatter(it, s=s, sig=sig):
            acc = ptab[pl.ds(pl.multiple_of((ACC + it * 64) * 8, 8), 128), :]
            for ck in range(1, 4):
                acc = acc + ptab[pl.ds(pl.multiple_of((ACC + it * 64 + ck * 16) * 8, 8), 128), :]
            acc = acc.reshape(16, 8, 128)
            l0 = 16 * it if s == 0 else sig * (128 + 16 * it)
            h0 = l0 // 2
            for j0 in range(16):
                v = acc[j0]
                v = v + swaph(v)
                if sig == 1:
                    box = (0,)
                elif j0 % 2 == 0:
                    box = tuple(range(-(sig // 2), sig // 2 + 1))
                else:
                    box = tuple(range(-(sig // 2) + 1, sig // 2))
                for dlt in box:
                    t_off = sig * j0 + dlt
                    st_k(t_off & 1, h0 + (t_off >> 1), v)
        with jax.named_scope('V_scatter'):
            jax.lax.fori_loop(0, nit, lambda it, c, scatter=scatter: (scatter(it), c)[1], 0)

        if s == 3:
            def body2048(np_, acc):
                return acc + ld(ptab, G_RE + 8 * 64 + np_)
            acc = jax.lax.fori_loop(0, 64, body2048, jnp.zeros((8, 128), F32), unroll=8)
            v = acc + swaph(acc)
            for t in range(2044, 2048):
                st_k(t & 1, t >> 1, v)

    for br in range(2):
        def fwd1(n2, br=br):
            xs = [(ld(pa, A_RE + 32 * n1 + n2), ld(pa, A_IM + 32 * n1 + n2)) for n1 in range(32)]
            if br == 1:
                xs2 = []
                for n1 in range(32):
                    wr, wi = tw(2 * (32 * n1 + n2))
                    xr, xi = xs[n1]
                    xs2.append((xr * wr - xi * wi, xr * wi + xi * wr))
                xs = xs2
            ys = _dft(xs, -1)
            for k1 in range(32):
                yr, yi = ys[k1]
                if k1 > 0:
                    wr, wi = tw(4 * k1 * n2)
                    yr, yi = yr * wr - yi * wi, yr * wi + yi * wr
                st(pb, B_RE + br * 1024 + k1 * 32 + n2, yr)
                st(pb, B_IM + br * 1024 + k1 * 32 + n2, yi)
        run_vpu('fwd1_%d' % br, fwd1, 32, 8)

    def fwd2(gk):
        br = gk // 32
        k1 = gk % 32
        xs = [(ld(pb, B_RE + gk * 32 + n2), ld(pb, B_IM + gk * 32 + n2)) for n2 in range(32)]
        ys = _dft(xs, -1)
        for k2 in range(32):
            k = 2 * (k1 + 32 * k2) + br
            st(pa, A_RE + k, ys[k2][0])
            st(pa, A_IM + k, ys[k2][1])
    run_vpu('fwd2', fwd2, 64, 8)

    M = 2048

    def post(j):
        for qq in range(8):
            k2 = jnp.minimum(8 * j + qq, 512)
            for par in range(2):
                k = 2 * k2 + par
                kb = (M - k) & (M - 1)
                ar, ai = ld(pa, A_RE + k), ld(pa, A_IM + k)
                br_, bi_ = ld(pa, A_RE + kb), ld(pa, A_IM + kb)
                wr, wi = tw(k)
                er = ar + br_
                ei = ai - bi_
                dr = ar - br_
                di = ai + bi_
                tr = wr * di + wi * dr
                ti = wi * di - wr * dr
                x1r, x1i = er + tr, ei + ti
                x2r, x2i = er - tr, ti - ei
                r1r, r1i = swaph(x1r), swaph(x1i)
                r2r, r2i = swaph(x2r), swaph(x2i)
                y1r = x1r * r1r - x1i * r1i
                y1i = x1r * r1i + x1i * r1r
                y2r = x2r * r2r - x2i * r2i
                y2i = x2r * r2i + x2i * r2r
                yer = y1r + y2r
                yei = y1i - y2i
                qr = y1r - y2r
                qi = y1i + y2i
                yor = qr * wr + qi * wi
                yoi = qi * wr - qr * wi
                z1r = yer - yoi
                z1i = yei + yor
                z2r = yer + yoi
                z2i = yor - yei
                q1 = k2
                q2 = (1024 - k2) if par == 0 else (1023 - k2)
                lo = 4 * par
                for q, vr, vi in ((q1, z1r, z1i), (q2, z2r, z2i)):
                    qq_ = jnp.where(q > 1023, 0, q) if par == 0 else q
                    pb[pl.ds(pl.multiple_of((B_RE + qq_) * 8, 8) + lo, 4), :] = vr[lo:lo + 4]
                    pb[pl.ds(pl.multiple_of((B_IM + qq_) * 8, 8) + lo, 4), :] = vi[lo:lo + 4]
    run_vpu('post', post, 72, 9)

    def inv1(n2):
        xs = [(ld(pb, B_RE + 32 * n1 + n2), ld(pb, B_IM + 32 * n1 + n2)) for n1 in range(32)]
        ys = _dft(xs, +1)
        for k1 in range(32):
            yr, yi = ys[k1]
            if k1 > 0:
                wr, wi = tw(4 * k1 * n2)
                wi = -wi
                yr, yi = yr * wr - yi * wi, yr * wi + yi * wr
            st(pa, A_RE + k1 * 32 + n2, yr)
            st(pa, A_IM + k1 * 32 + n2, yi)
    run_vpu('inv1', inv1, 32, 8)

    def inv2(k1):
        xs = [(ld(pa, A_RE + k1 * 32 + n2), ld(pa, A_IM + k1 * 32 + n2)) for n2 in range(32)]
        ys = _dft(xs, +1)
        for k2 in range(32):
            st(pb, B_RE + k1 + 32 * k2, ys[k2][0])
            st(pb, B_IM + k1 + 32 * k2, ys[k2][1])
    run_vpu('inv2', inv2, 32, 8)

    def comb(j):
        for qq in range(32):
            m = 32 * j + qq
            vr, vi = ld(pb, B_RE + m), ld(pb, B_IM + m)
            wr, wi = tw(2 * m)
            wi = -wi
            rr, ri = swaph(vr), swaph(vi)
            st(pa, A_RE + m, vr + (rr * wr - ri * wi))
            st(pa, A_IM + m, vi + (rr * wi + ri * wr))
    run_vpu('comb', comb, 32, 8)

    def y_out(jj):
        for qq in range(4):
            j = 4 * jj + qq
            for g in range(4):
                ev = pa[pl.ds((A_RE + 8 * j) * 8 + g, 8, stride=8), :]
                od = pa[pl.ds((A_IM + 8 * j) * 8 + g, 8, stride=8), :]
                ybuf[pl.ds(g * L + 16 * j, 8, stride=2), :] = ev
                ybuf[pl.ds(g * L + 16 * j + 1, 8, stride=2), :] = od
        r0 = pl.multiple_of(64 * jj, 64)
        for g in range(4):
            dsk = dsk_ref[:, 128 * g:128 * (g + 1)].astype(F32)
            yb = ybuf[pl.ds(g * L + r0, 64), :].astype(BF16).astype(F32)
            sk = (ubuf[pl.ds(g * L + r0, 64), :] * dsk).astype(BF16).astype(F32)
            o_ref[pl.ds(r0, 64), 512 + 128 * g:512 + 128 * (g + 1)] = (yb + sk).astype(BF16)
    run_vpu('yout', y_out, 32, 16)
    out_b.start()

    flush_mxu()
    cp_wo.wait()
    with jax.named_scope('M_o'):
        for j in range(S // QRB):
            o_unit(j)
    out_b.wait()
    for j in range(S // QRB):
        out_a(j).wait()


@jax.jit
def pallas_concat_heads__sliding_block__ssm_conv_s4__prompt_kernel(
    A_x: jax.Array,
    A_wqkv: jax.Array,
    A_wo: jax.Array,
    B_u: jax.Array,
    B_A_re: jax.Array,
    B_A_im: jax.Array,
    B_B_re: jax.Array,
    B_B_im: jax.Array,
    B_C_re: jax.Array,
    B_C_im: jax.Array,
    B_log_dt: jax.Array,
    B_Dskip: jax.Array,
):
    vm = pl.BlockSpec(memory_space=pltpu.VMEM)
    hbm = pl.BlockSpec(memory_space=pl.ANY)
    out = pl.pallas_call(
        _kernel,
        out_shape=jax.ShapeDtypeStruct((S, 2 * D), BF16),
        in_specs=[pl.BlockSpec(memory_space=pltpu.SMEM)] + [hbm] * 4 + [vm] * 8,
        out_specs=hbm,
        scratch_shapes=[
            pltpu.VMEM((S, D), BF16),
            pltpu.VMEM((32 * NKB * 128, 128), BF16),
            pltpu.VMEM((32 * 32, 256 + S), BF16),
            pltpu.VMEM((D, S), BF16),
            pltpu.VMEM((4096 * 8, 128), F32),
            pltpu.VMEM((4096 * 8, 128), F32),
            pltpu.VMEM((NSEED * 8, 128), F32),
            pltpu.VMEM((NTAB * 8, 128), F32),
            pltpu.VMEM((384 * 8, 128), F32),
            pltpu.VMEM((4 * L, 128), F32),
            pltpu.VMEM((4 * L, 128), F32),
            pltpu.VMEM((S, D), BF16),
            pltpu.VMEM((D, 3 * D), BF16),
            pltpu.VMEM((D, D), BF16),
            pltpu.VMEM((L, D), BF16),
            pltpu.VMEM((S, 2 * D), BF16),
            pltpu.SemaphoreType.DMA((4,)),
            pltpu.SemaphoreType.DMA((1 + S // QRB,)),
        ],
        compiler_params=pltpu.CompilerParams(vmem_limit_bytes=120 * 1024 * 1024),
    )(jnp.asarray(_tw_table()), A_x.reshape(S, D), A_wqkv, A_wo, B_u.reshape(L, D),
      B_A_re, B_A_im, B_B_re, B_B_im, B_C_re, B_C_im, B_log_dt.reshape(4, 128), B_Dskip.reshape(1, D))
    return out.reshape(1, S, 2 * D)
```
